```python
import jax
import jax.numpy as jnp

def _softmax(x, axis=-1):
    return jax.nn.softmax(x, axis=axis)
def _gelu(x):
    return jax.nn.gelu(x, approximate=True)
def _silu(x):
    return jax.nn.silu(x)
def _sigmoid(x):
    return jax.nn.sigmoid(x)
def _layernorm(x, axis=-1, eps=1e-5):
    m = jnp.mean(x, axis=axis, keepdims=True)
    v = jnp.var(x, axis=axis, keepdims=True)
    return (x - m) / jnp.sqrt(v + eps)
def _scatter_add(tgt, idx, src, axis=0):
    return tgt.at[idx].add(src)
def _segment_sum(src, seg, n):
    return jax.ops.segment_sum(src, seg, n)
class _Rng:
    def __init__(self, key):
        self._k = key
    def _next(self):
        self._k, sub = jax.random.split(self._k)
        return sub
    def normal(self, shape):
        return jax.random.normal(self._next(), shape, dtype=jnp.bfloat16)
    def randint(self, lo, hi, shape):
        return jax.random.randint(self._next(), shape, lo, hi, dtype=jnp.int32)
    def uniform(self, shape, lo=0.0, hi=1.0):
        return jax.random.uniform(self._next(), shape, jnp.bfloat16, lo, hi)
    def permutation(self, n):
        return jax.random.permutation(self._next(), n)


kernel_name = 'interleave_layers__sliding_block_cached__glu_gated_swiglu__decode'

def setup_inputs():
    _rng = _Rng(jax.random.key(int.from_bytes(__import__("os").urandom(4), "little")))
    _w = (lambda a: (lambda t: t.astype(jnp.bfloat16) if jnp.issubdtype(t.dtype, jnp.floating) else t)(jnp.asarray(a)))
    def _A_setup():
        B, Sq, D = 1, 1, 640
        Hq, Hkv, Sk, Dh = 32, 32, 32768, 192
        assert Hq % Hkv == 0, (Hq, Hkv)
        return {
            "x": _w((lambda *s: _rng.normal(s) * 0.05)(B, Sq, D)),
            "k_cache": _w((lambda *s: _rng.normal(s) * 0.05)(B, Hkv, Sk, Dh)),
            "v_cache": _w((lambda *s: _rng.normal(s) * 0.05)(B, Hkv, Sk, Dh)),
            "wq": _w((lambda *s: _rng.normal(s) * 0.05)(D, Hq * Dh) * (D ** -0.5)),
            "wo": _w((lambda *s: _rng.normal(s) * 0.05)(Hq * Dh, D) * ((Hq * Dh) ** -0.5)),
        }
    _A_in = _A_setup()

    def _B_setup():
        B, S, D, F = 1, 1, 640, 1536
        return {
            "x": _w((lambda *s: _rng.normal(s) * 0.05)(B, S, D)),
            "w1": _w((lambda *s: _rng.normal(s) * 0.05)(D, F) * (2.0 / D) ** 0.5),
            "w3": _w((lambda *s: _rng.normal(s) * 0.05)(D, F) * (2.0 / D) ** 0.5),
            "w2": _w((lambda *s: _rng.normal(s) * 0.05)(F, D) * (2.0 / F) ** 0.5),
        }
    _B_in = _B_setup()

    return {
        "A_x": _A_in["x"],
        "A_k_cache": _A_in["k_cache"],
        "A_v_cache": _A_in["v_cache"],
        "A_wq": _A_in["wq"],
        "A_wo": _A_in["wo"],
        "B_x": _B_in["x"],
        "B_w1": _B_in["w1"],
        "B_w3": _B_in["w3"],
        "B_w2": _B_in["w2"],
    }

def reference(A_x, A_k_cache, A_v_cache, A_wq, A_wo, B_x, B_w1, B_w3, B_w2):
    def _A_ref(x, k_cache, v_cache, wq, wo):
        B, Sq, D = x.shape
        Hq, Dh = 32, 192
        Hkv, Sk = k_cache.shape[1], k_cache.shape[2]
        W = min(4096, max(256, Sk // 4))
        rep = Hq // Hkv
        q = (lambda x, *d: x.transpose(*d))((x @ wq).reshape(B, Sq, Hq, Dh), 0, 2, 1, 3)
        k = jnp.repeat(k_cache[:, :, Sk - W:, :], rep, axis=1)
        v = jnp.repeat(v_cache[:, :, Sk - W:, :], rep, axis=1)
        scores = jnp.einsum("bhqd,bhkd->bhqk", q, k) * (Dh ** -0.5)
        p = _softmax(scores, axis=-1)
        o = jnp.einsum("bhqk,bhkd->bhqd", p, v)
        return (lambda x, *d: x.transpose(*d))(o, 0, 2, 1, 3).reshape(B, Sq, Hq * Dh) @ wo

    def _B_ref(x, w1, w3, w2):
        gate = jnp.einsum("bsd,df->bsf", x, w1)
        up = jnp.einsum("bsd,df->bsf", x, w3)
        h = _silu(gate) * up
        out = jnp.einsum("bsf,fd->bsd", h, w2)
        return out

    x = A_x
    x = x + _A_ref(_layernorm(x, axis=-1), A_k_cache, A_v_cache, A_wq, A_wo)
    x = x + _B_ref(_layernorm(x, axis=-1), B_w1, B_w3, B_w2)
    x = x + _A_ref(_layernorm(x, axis=-1), A_k_cache, A_v_cache, A_wq, A_wo)
    x = x + _B_ref(_layernorm(x, axis=-1), B_w1, B_w3, B_w2)
    return x
```

```python
import functools

import jax
import jax.numpy as jnp
import numpy as np
from jax import lax
import jax.experimental.pallas as pl
import jax.experimental.pallas.tpu as pltpu

F32, BF16, U32 = jnp.float32, jnp.bfloat16, jnp.uint32

D = 640
H = 32
DH = 192
SK = 32768
W = min(4096, max(256, SK // 4))
FF = 1536
NP = H // 2
NKT = W // 128
NQ = NKT // 4
ND = D // 128
NF = FF // 128
GP = 2 * DH // 16
EXP2_SCALE = float(DH ** -0.5 * np.log2(np.e))
EPS = 1e-5


def _mm(a, b):
    return lax.dot_general(a, b, (((1,), (0,)), ((), ())),
                           precision=lax.Precision.DEFAULT,
                           preferred_element_type=F32)


def _rnd(a):
    return a.astype(BF16).astype(F32)


def _tile(ref, g0, ng, c):
    return pltpu.bitcast(ref[pl.ds(g0, ng), c].reshape(ng * 8, 128), BF16)


def _allsum_rows(a):
    a = a + pltpu.roll(a, 4, 0)
    a = a + pltpu.roll(a, 2, 0)
    return a + pltpu.roll(a, 1, 0)


def _layernorm(x):
    m = jnp.sum(x, axis=1, keepdims=True) * (1.0 / D)
    xc = x - m
    v = jnp.sum(xc * xc, axis=1, keepdims=True) * (1.0 / D)
    return _rnd(_rnd(x - _rnd(m)) / _rnd(jnp.sqrt(_rnd(_rnd(v) + EPS))))


def make_kernel(mxq=1, mxq_last=5, dma=True, layers=2, order=0):
    def kernel(x_hbm, k_hbm, v_hbm, wq_hbm, wo_hbm, w1_hbm, w3_hbm, w2_hbm, o_ref,
               xb, kb, vb, wqb, wob, w1b, w3b, w2b, qs, ps, ls, accs, sem_kv, sem_w):
        kr, vr = kb.bitcast(U32), vb.bitcast(U32)
        wqr, wor = wqb.bitcast(U32), wob.bitcast(U32)
        w1r, w3r, w2r = w1b.bitcast(U32), w3b.bitcast(U32), w2b.bitcast(U32)

        def kv_copies(which, i):
            src, dst = ((k_hbm, kb), (v_hbm, vb))[which]
            return [pltpu.make_async_copy(
                src.at[pl.ds(i * GP, GP), half, pl.ds((SK - W) // 128, NKT)],
                dst.at[pl.ds(i * GP, GP), :, pl.ds(half * 8, 8)],
                sem_kv.at[which, i, half]) for half in range(2)]

        def w_copies(j):
            src, dst = ((wq_hbm, wqb), (wo_hbm, wob), (w1_hbm, w1b), (w3_hbm, w3b),
                        (w2_hbm, w2b))[j]
            return [pltpu.make_async_copy(
                src.at[:, half], dst.at[:, :, pl.ds(half * 8, 8)], sem_w.at[j, half])
                for half in range(2)]

        def start(cps):
            if dma:
                for c in cps:
                    c.start()

        def wait(cps):
            if dma:
                for c in cps:
                    c.wait()

        x_copy = pltpu.make_async_copy(x_hbm, xb, sem_w.at[5, 0])
        x_copy.start()
        start(w_copies(0))
        start(kv_copies(0, 0))
        start(w_copies(1))
        for i in range(3):
            start(kv_copies(0, i + 1))
            start(kv_copies(1, i))
        x_copy.wait()

        row = lax.broadcasted_iota(jnp.int32, (8, 128), 0)
        lane = lax.broadcasted_iota(jnp.int32, (8, 128), 1)
        head_of_lane = [jnp.zeros_like(lane), (lane >= 64).astype(jnp.int32),
                        jnp.ones_like(lane)]
        head_mask = [(row & 1) == h for h in head_of_lane]
        slot_mask = [(row >> 1) == s for s in range(4)]

        def q_proj(ln, i):
            for dt in range(3):
                q = _mm(ln, _tile(wqr, 0, D // 16, i * 3 + dt))
                qs[i, dt] = jnp.where(head_mask[dt], _rnd(q), 0.0)

        def scores(i):
            q = [qs[i, dt] for dt in range(3)]
            lhs = [jnp.concatenate([jnp.where(slot_mask[s], q[dt], 0.0) for dt in range(3)],
                                   axis=1) for s in range(4)]
            out = []
            for j in range(NQ):
                parts = [_mm(lhs[s], _tile(kr, i * GP, GP, 4 * j + s)) for s in range(4)]
                out.append((parts[0] + parts[1]) + (parts[2] + parts[3]))
            return out

        def softmax(s, buf):
            m = functools.reduce(jnp.maximum, s)
            m = jnp.broadcast_to(jnp.max(m, axis=1, keepdims=True), (8, 128))
            m = jnp.maximum(m, pltpu.roll(m, 4, 0))
            m = jnp.maximum(m, pltpu.roll(m, 2, 0))
            l = None
            for j in range(NQ):
                p = jnp.exp2((s[j] - m) * EXP2_SCALE)
                ps[buf, j] = p
                l = p if l is None else l + p
            ls[buf] = l

        def transpose_v(i, nq):
            def body(c, carry):
                for dt in range(3):
                    g0 = i * GP + dt * 8
                    t = pltpu.bitcast(_tile(vr, g0, 8, c).T, U32)
                    vr[pl.ds(g0, 8), c] = t.reshape(8, 8, 128)
                return carry
            lax.fori_loop(NKT - 4 * nq, NKT, body, 0)

        def pv(i, buf, nq):
            for hh in range(2):
                lo = [None] * 12
                hi = [None] * 12
                for c in range(NKT - 4 * nq):
                    r = (c % 4) * 2 + hh
                    p = jnp.broadcast_to(ps[buf, c // 4, pl.ds(r, 1), :], (8, 128))
                    for g in range(12):
                        w = vr[i * GP + hh * 12 + g, c]
                        a = pltpu.bitcast(w << 16, F32) * p
                        b = pltpu.bitcast(w & np.uint32(0xFFFF0000), F32) * p
                        lo[g] = a if lo[g] is None else lo[g] + a
                        hi[g] = b if hi[g] is None else hi[g] + b
                for g in range(12):
                    r0 = (hh * 12 + g) * 16
                    accs[pl.ds(r0, 8, stride=2), :] = lo[g]
                    accs[pl.ds(r0 + 1, 8, stride=2), :] = hi[g]
            om = [None] * 3
            for j in range(NQ - nq, NQ):
                p = _rnd(ps[buf, j])
                for s in range(4):
                    lhs = jnp.where(slot_mask[s], p, 0.0)
                    for dt in range(3):
                        t = _mm(lhs, _tile(vr, i * GP + dt * 8, 8, 4 * j + s))
                        om[dt] = t if om[dt] is None else om[dt] + t
            l = jnp.broadcast_to(jnp.sum(ls[buf], axis=1, keepdims=True), (8, 128))
            l = l + pltpu.roll(l, 4, 0)
            l = l + pltpu.roll(l, 2, 0)
            inv = 1.0 / l
            inv_other = pltpu.roll(inv, 1, 0)
            o = []
            for dt in range(3):
                t = accs[pl.ds(dt * 128, 128), :].T.reshape(16, 8, 128)
                t = jnp.sum(t, axis=0)
                if nq:
                    t = t + jnp.where(head_mask[dt], om[dt], 0.0)
                t = _allsum_rows(t)
                o.append(_rnd(t * jnp.where(head_mask[dt], inv, inv_other)))
            return jnp.concatenate(o, axis=1)

        def out_proj(o, i, y):
            return jnp.concatenate(
                [y[:, ct * 128:(ct + 1) * 128] + _mm(o, _tile(wor, i * GP, GP, ct))
                 for ct in range(ND)], axis=1)

        def layer(li, x):
            first = li == 0
            ln = _layernorm(x)

            @pl.when(first)
            def _():
                wait(w_copies(0))
                wait(kv_copies(0, 0))
                wait(w_copies(1))

            q_proj(ln, 0)
            q_proj(ln, 1)
            softmax(scores(0), 0)

            def step(i, carry):
                o_prev, y = carry

                @pl.when(first)
                def _():
                    @pl.when(i + 4 < NP)
                    def _():
                        start(kv_copies(0, i + 4))

                    @pl.when(i + 3 < NP)
                    def _():
                        start(kv_copies(1, i + 3))

                    @pl.when(i + 3 == NP)
                    def _():
                        for j in (2, 3, 4):
                            start(w_copies(j))

                    wait(kv_copies(0, i + 1))
                    wait(kv_copies(1, i))
                    if mxq:
                        transpose_v(i, mxq)

                buf = i & 1
                if order == 0:
                    s = scores(i + 1)
                    o = pv(i, buf, mxq)
                    softmax(s, 1 - buf)
                    q_proj(ln, jnp.minimum(i + 2, NP - 1))
                    y = out_proj(o_prev, jnp.maximum(i - 1, 0), y)
                else:
                    o = pv(i, buf, mxq)
                    s = scores(i + 1)
                    softmax(s, 1 - buf)
                    q_proj(ln, jnp.minimum(i + 2, NP - 1))
                    y = out_proj(o_prev, jnp.maximum(i - 1, 0), y)
                return o, y

            o_prev, y = lax.fori_loop(
                0, NP - 1, step, (jnp.zeros((8, 384), F32), jnp.zeros((8, D), F32)))

            @pl.when(first)
            def _():
                wait(kv_copies(1, NP - 1))
                transpose_v(NP - 1, mxq_last)

            y = out_proj(o_prev, NP - 2, y)
            o = pv(NP - 1, (NP - 1) & 1, mxq_last)
            y = out_proj(o, NP - 1, y)
            x = _rnd(x + _rnd(y))

            ln = _layernorm(x)

            @pl.when(first)
            def _():
                wait(w_copies(2))
                wait(w_copies(3))

            hs = []
            for ft in range(NF):
                gate = _rnd(_mm(ln, _tile(w1r, 0, D // 16, ft)))
                up = _rnd(_mm(ln, _tile(w3r, 0, D // 16, ft)))
                hs.append(_rnd(_rnd(gate * (1.0 / (1.0 + jnp.exp(-gate)))) * up))
            h = jnp.concatenate(hs, axis=1)

            @pl.when(first)
            def _():
                wait(w_copies(4))

            f = jnp.concatenate([_mm(h, _tile(w2r, 0, FF // 16, ct)) for ct in range(ND)],
                                axis=1)
            return _rnd(x + _rnd(f))

        x = jnp.broadcast_to(xb[...].astype(F32), (8, D))
        x = lax.fori_loop(0, layers, layer, x)
        o_ref[...] = x[0:1].astype(BF16)

    return kernel


def _tiles(a):
    r, c = a.shape
    return a.reshape(r // 16, 2, 8, c // 128, 128).transpose(0, 1, 3, 2, 4)


def _cache_tiles(a):
    a = a.reshape(H, SK // 128, 128, DH // 8, 8).transpose(0, 3, 1, 4, 2)
    return a.reshape(H * DH // 16, 2, SK // 128, 8, 128)


def build(name="fused", flags=None, **kw):
    @jax.jit
    def fn(A_x, A_k_cache, A_v_cache, A_wq, A_wo, B_x, B_w1, B_w3, B_w2):
        del B_x
        hbm = pl.BlockSpec(memory_space=pl.ANY)
        out = pl.pallas_call(
            make_kernel(**kw),
            out_shape=jax.ShapeDtypeStruct((1, D), BF16),
            in_specs=[hbm] * 8,
            out_specs=pl.BlockSpec(memory_space=pltpu.VMEM),
            scratch_shapes=[
                pltpu.VMEM((1, D), BF16),
                pltpu.VMEM((NP * GP, NKT, 16, 128), BF16),
                pltpu.VMEM((NP * GP, NKT, 16, 128), BF16),
                pltpu.VMEM((D // 16, H * DH // 128, 16, 128), BF16),
                pltpu.VMEM((H * DH // 16, ND, 16, 128), BF16),
                pltpu.VMEM((D // 16, NF, 16, 128), BF16),
                pltpu.VMEM((D // 16, NF, 16, 128), BF16),
                pltpu.VMEM((FF // 16, ND, 16, 128), BF16),
                pltpu.VMEM((NP, 3, 8, 128), F32),
                pltpu.VMEM((2, NQ, 8, 128), F32),
                pltpu.VMEM((2, 8, 128), F32),
                pltpu.VMEM((2 * DH, 128), F32),
                pltpu.SemaphoreType.DMA((2, NP, 2)),
                pltpu.SemaphoreType.DMA((6, 2)),
            ],
            compiler_params=pltpu.CompilerParams(
                vmem_limit_bytes=124 * 1024 * 1024, flags=flags),
            name=name,
        )(A_x.reshape(1, D), _cache_tiles(A_k_cache), _cache_tiles(A_v_cache),
          _tiles(A_wq), _tiles(A_wo), _tiles(B_w1), _tiles(B_w3), _tiles(B_w2))
        return out.reshape(1, 1, D)
    return fn


pallas_interleave_layers__sliding_block_cached__glu_gated_swiglu__decode_kernel = build()
```

```python
import functools
import itertools

import jax
import jax.numpy as jnp
import numpy as np
from jax import lax
import jax.experimental.pallas as pl
import jax.experimental.pallas.tpu as pltpu

F32, BF16, U32 = jnp.float32, jnp.bfloat16, jnp.uint32

D = 640
H = 32
DH = 192
SK = 32768
W = min(4096, max(256, SK // 4))
FF = 1536
NP = H // 2
NKT = W // 128
NQ = NKT // 4
ND = D // 128
NF = FF // 128
GP = 2 * DH // 16
NB = 3
AHEAD = 3
EXP2_SCALE = float(DH ** -0.5 * np.log2(np.e))
EPS = 1e-5


def _mm(a, b):
    return lax.dot_general(a, b, (((1,), (0,)), ((), ())),
                           precision=lax.Precision.DEFAULT,
                           preferred_element_type=F32)


def _rnd(a):
    return a.astype(BF16).astype(F32)


def _tile(ref, g0, c):
    return pltpu.bitcast(ref[pl.ds(g0, 8), c].reshape(64, 128), BF16)


def _allsum_rows(a):
    a = a + pltpu.roll(a, 4, 0)
    a = a + pltpu.roll(a, 2, 0)
    return a + pltpu.roll(a, 1, 0)


def _lane_sum(tiles):
    s = jnp.sum(functools.reduce(jnp.add, tiles), axis=1, keepdims=True)
    return jnp.broadcast_to(s, (8, 128))


def _layernorm(x):
    m = _lane_sum(x) * (1.0 / D)
    v = _lane_sum([(t - m) * (t - m) for t in x]) * (1.0 / D)
    r = lax.rsqrt(v + EPS)
    return [_rnd((t - m) * r) for t in x]


def _run(*gens):
    for g in gens:
        for _ in g:
            pass


def _interleave(a, b, ratio, every, fence):
    end = object()
    ta = tb = 0.0
    nxt = every
    while a is not None or b is not None:
        if a is not None and b is not None and tb >= nxt:
            fence()
            nxt = tb + every
        if b is None or (a is not None and ta * ratio <= tb):
            c = next(a, end)
            if c is end:
                a = None
            else:
                ta += c
        else:
            c = next(b, end)
            if c is end:
                b = None
            else:
                tb += c


def make_kernel(mxc=4, mxc_last=16, dma=True, layers=2, ratio=0.97, gblk=2, every=128,
                lag_v=0, tie=2, lag_f=36, lag_m=18, smw=20, offset=0, ratio_last=0.85, cv=1.5, ncs=(4, 4, 4)):

    def kernel(x_hbm, k_hbm, v_hbm, wq_hbm, wo_hbm, w1_hbm, w3_hbm, w2_hbm, o_ref,
               kvb, wqb, wob, w1b, w3b, w2b, qs, ss, *rest):
        ps, accs, (xb, sem_kv, sem_w) = rest[:NB], rest[NB:2 * NB], rest[2 * NB:]
        kvr = pltpu.annotate(kvb, no_hazard=True).bitcast(U32)
        wqr, wor = wqb.bitcast(U32), wob.bitcast(U32)
        w1r, w3r, w2r = w1b.bitcast(U32), w3b.bitcast(U32), w2b.bitcast(U32)

        def kv_copies(which, i, slot):
            src = (k_hbm, v_hbm)[which]
            return [pltpu.make_async_copy(
                src.at[pl.ds(i * GP, GP), half, pl.ds((SK - W) // 128, NKT)],
                kvb.at[pl.ds((which * NP + i) * GP, GP), :, pl.ds(half * 8, 8)],
                sem_kv.at[slot]) for half in range(2)]

        def step_copies(i):
            slot = i & 3
            return kv_copies(0, i + 1, slot) + kv_copies(1, i, slot)

        def w_copies(j, slot):
            src, dst = ((wq_hbm, wqb), (wo_hbm, wob), (w1_hbm, w1b), (w3_hbm, w3b),
                        (w2_hbm, w2b))[j]
            return [pltpu.make_async_copy(
                src.at[:, half], dst.at[:, :, pl.ds(half * 8, 8)], sem_w.at[slot])
                for half in range(2)]

        first_copies = lambda: w_copies(0, 0) + kv_copies(0, 0, 4) + w_copies(1, 0)
        last_copies = lambda: kv_copies(1, NP - 1, 4)
        up_copies = lambda: w_copies(2, 1) + w_copies(3, 1)
        down_copies = lambda: w_copies(4, 0)

        def start(cps):
            if dma:
                for c in cps:
                    c.start()

        def wait(cps):
            if dma:
                for c in cps:
                    c.wait()

        x_copy = pltpu.make_async_copy(x_hbm, xb, sem_w.at[1])
        x_copy.start()
        start(first_copies())
        for i in range(AHEAD):
            start(step_copies(i))
        x_copy.wait()
        x = jnp.broadcast_to(xb[...].astype(F32), (8, D))
        x = [x[:, c * 128:(c + 1) * 128] for c in range(ND)]

        row = lax.broadcasted_iota(jnp.int32, (8, 128), 0)
        lane = lax.broadcasted_iota(jnp.int32, (8, 128), 1)
        head_of_lane = [jnp.zeros_like(lane), (lane >= 64).astype(jnp.int32),
                        jnp.ones_like(lane)]
        head_mask = [(row & 1) == h for h in head_of_lane]
        slot_mask = [(row >> 1) == s for s in range(4)]

        spot = jnp.max(pltpu.bitcast(x[0], jnp.int32) & 1)
        never = lane == spot + 128
        hist = {}

        def reset():
            hist.update(vpu=[], mxu=[], due=[], n=0)

        def fence():
            if len(hist["mxu"]) > lag_m:
                kvr[2 * NP * GP, spot] = pltpu.bitcast(hist["mxu"][-1 - lag_m], U32)

        def tied(a):
            hist["n"] += 1
            if hist["due"] and hist["due"][0][0] <= hist["n"]:
                return jnp.where(never, hist["due"].pop(0)[1], a)
            if hist["n"] % tie == 0 and len(hist["vpu"]) > lag_v:
                live = hist["vpu"][-1 - lag_v]
                return jnp.where(never, live[(hist["n"] // tie) % len(live)], a)
            return a

        def mm(a, b, mask=None):
            a = tied(a)
            t = _mm(a if mask is None else jnp.where(mask, a, 0.0), b)
            hist["mxu"].append(t)
            return t

        def matvec(a, ref, g0, cols, out):
            for n, c in enumerate(cols):
                for kt, at in enumerate(a):
                    t = mm(at, _tile(ref, g0 + kt * 8, c))
                    out[n] = t if out[n] is None else out[n] + t
                    yield 8

        def q_proj(ln, i):
            q = [None] * 3
            yield from matvec(ln, wqr, 0, [i * 3 + dt for dt in range(3)], q)
            for dt in range(3):
                qs[i, dt] = jnp.where(head_mask[dt], _rnd(q[dt]), 0.0)

        def scores(i, buf, meanwhile=()):
            q = [qs[i, dt] for dt in range(3)]
            m = None
            for j in range(NQ):
                s = None
                for sl in range(4):
                    for dt in range(3):
                        t = mm(q[dt], _tile(kvr, i * GP + dt * 8, 4 * j + sl), slot_mask[sl])
                        s = t if s is None else s + t
                        yield 8
                ss[j] = s
                m = s if m is None else jnp.maximum(m, s)
            m = jnp.broadcast_to(jnp.max(m, axis=1, keepdims=True), (8, 128))
            m = jnp.maximum(m, pltpu.roll(m, 4, 0))
            m = jnp.maximum(m, pltpu.roll(m, 2, 0))
            yield from meanwhile
            l = None
            for j in range(NQ):
                p = jnp.exp2((ss[j] - m) * EXP2_SCALE)
                ps[buf][j] = p
                l = p if l is None else l + p
            ps[buf][NQ] = l

        def transpose_v(i, nc):
            def body(c, carry):
                for dt in range(3):
                    g0 = (NP + i) * GP + dt * 8
                    t = pltpu.bitcast(_tile(kvr, g0, c).T, U32)
                    kvr[pl.ds(g0, 8), c] = t.reshape(8, 8, 128)
                return carry
            lax.fori_loop(NKT - nc, NKT, body, 0)

        def pv_vpu(i, buf, nc, side=iter(())):
            for hh in range(2):
                for gb in range(0, 12, gblk):
                    yield next(side, 0)
                    lo = [None] * gblk
                    hi = [None] * gblk
                    for c in range(NKT - nc):
                        p = ps[buf][c // 4, pl.ds((c % 4) * 2 + hh, 8, stride=0), :]
                        for g in range(gblk):
                            w = kvr[(NP + i) * GP + hh * 12 + gb + g, c]
                            a = pltpu.bitcast(w << 16, F32) * p
                            b = pltpu.bitcast(w & np.uint32(0xFFFF0000), F32) * p
                            lo[g] = a if lo[g] is None else lo[g] + a
                            hi[g] = b if hi[g] is None else hi[g] + b
                            yield cv
                        hist["vpu"].append(lo + hi)
                    for g in range(gblk):
                        r0 = (hh * 12 + gb + g) * 16
                        accs[buf][pl.ds(r0, 8, stride=2), :] = lo[g]
                        accs[buf][pl.ds(r0 + 1, 8, stride=2), :] = hi[g]

        def pv_mxu(i, buf, nc, om):
            for c in range(NKT - nc, NKT):
                p = _rnd(ps[buf][c // 4])
                for dt in range(3):
                    t = mm(p, _tile(kvr, (NP + i) * GP + dt * 8, c), slot_mask[c % 4])
                    om[dt] = t if om[dt] is None else om[dt] + t
                    yield 8

        def pv_finish(buf, om, o):
            l = _lane_sum([ps[buf][NQ]])
            l = l + pltpu.roll(l, 4, 0)
            l = l + pltpu.roll(l, 2, 0)
            inv = 1.0 / l
            inv_other = pltpu.roll(inv, 1, 0)
            for dt in range(3):
                t = accs[buf][pl.ds(dt * 128, 128), :].T.reshape(16, 8, 128)
                t = jnp.sum(t, axis=0) + jnp.where(head_mask[dt], om[dt], 0.0)
                t = _allsum_rows(t)
                o[dt] = _rnd(t * jnp.where(head_mask[dt], inv, inv_other))
                hist["due"].append((hist["n"] + lag_f, o[dt]))
                yield 8

        def out_proj(o, i, y):
            return matvec(o, wor, i * GP, range(ND), y)

        def attention_streaming(ln):
            wait(first_copies())
            lax.fori_loop(0, NP, lambda i, c: _run(q_proj(ln, i)), None)
            reset()
            _run(scores(0, 0))

            def attend(i, nc, y):
                reset()
                transpose_v(i, nc)
                om, o, y = [None] * 3, [None] * 3, list(y)
                _run(pv_mxu(i, 0, nc, om), pv_vpu(i, 0, nc), pv_finish(0, om, o))
                reset()
                _run(out_proj(o, i, y))
                return y

            def step(i, y):
                @pl.when(i + AHEAD < NP - 1)
                def _():
                    start(step_copies(i + AHEAD))

                @pl.when(i + AHEAD == NP - 1)
                def _():
                    start(last_copies() + up_copies() + down_copies())

                wait(step_copies(i))
                y = attend(i, mxc, y)
                _run(scores(i + 1, 0))
                return y

            y = lax.fori_loop(0, NP - 1, step, [jnp.zeros((8, 128), F32)] * ND)
            wait(last_copies())
            return attend(NP - 1, mxc_last, y)

        def attention_resident(ln):
            reset()
            accs[NB - 1][...] = jnp.zeros((2 * DH, 128), F32)
            ps[NB - 1][NQ] = jnp.ones((8, 128), F32)
            _run(q_proj(ln, 0), scores(0, 0, q_proj(ln, 1)))

            def step(t, carry):
                om_prev, y = carry
                y = list(y)
                reset()
                ma, va = [], [iter([offset])]
                for u in range(NB):
                    i = t * NB + u
                    om, o = [None] * 3, [None] * 3
                    rest = itertools.chain(
                        pv_mxu(i, u, ncs[u], om), q_proj(ln, jnp.minimum(i + 2, NP - 1)),
                        out_proj(o, jnp.maximum(i - 1, 0), y))
                    ma += [scores(i + 1, (u + 1) % NB, itertools.islice(rest, smw)), rest]
                    va += [pv_vpu(i, u, ncs[u], pv_finish((u - 1) % NB, om_prev, o))]
                    om_prev = om
                _interleave(itertools.chain(*ma), itertools.chain(*va), ratio, every, fence)
                return om_prev, y

            zero = jnp.zeros((8, 128), F32)
            om_prev, y = lax.fori_loop(0, (NP - 1) // NB, step, ([zero] * 3, [zero] * ND))
            y = list(y)
            reset()
            om, o = [None] * 3, [None] * 3
            _interleave(
                itertools.chain(pv_mxu(NP - 1, 0, mxc_last, om), out_proj(o, NP - 2, y)),
                pv_vpu(NP - 1, 0, mxc_last, pv_finish(NB - 1, om_prev, o)),
                ratio_last, every, fence)
            o = [None] * 3
            _run(pv_finish(0, om, o))
            reset()
            _run(out_proj(o, NP - 1, y))
            return y

        def ffn(ln, first):
            if first:
                wait(up_copies())
            reset()
            h = []
            for ft in range(NF):
                gate, up = [None], [None]
                _run(matvec(ln, w1r, 0, [ft], gate), matvec(ln, w3r, 0, [ft], up))
                h.append(_rnd(gate[0] / (1.0 + jnp.exp(-gate[0])) * up[0]))
            if first:
                wait(down_copies())
            f = [None] * ND
            _run(*[matvec([h[kt]], w2r, kt * 8, range(ND), f) for kt in range(NF)])
            return f

        def add(x, y):
            return [_rnd(a + b) for a, b in zip(x, y)]

        def resident_layer(_, x):
            x = add(x, attention_resident(_layernorm(x)))
            return add(x, ffn(_layernorm(x), False))

        if dma:
            reset()
            x = add(x, attention_streaming(_layernorm(x)))
            x = add(x, ffn(_layernorm(x), True))
            x = resident_layer(0, x)
        else:
            x = lax.fori_loop(0, layers, resident_layer, x)
        o_ref[...] = jnp.concatenate(x, axis=1)[0:1].astype(BF16)

    return kernel


def _tiles(a):
    r, c = a.shape
    return a.reshape(r // 16, 2, 8, c // 128, 128).transpose(0, 1, 3, 2, 4)


def _cache_tiles(a):
    a = a.reshape(H, SK // 128, 128, DH // 8, 8).transpose(0, 3, 1, 4, 2)
    return a.reshape(H * DH // 16, 2, SK // 128, 8, 128)


def build(name="fused", flags=None, **kw):
    @jax.jit
    def fn(A_x, A_k_cache, A_v_cache, A_wq, A_wo, B_x, B_w1, B_w3, B_w2):
        del B_x
        hbm = pl.BlockSpec(memory_space=pl.ANY)
        out = pl.pallas_call(
            make_kernel(**kw),
            out_shape=jax.ShapeDtypeStruct((1, D), BF16),
            in_specs=[hbm] * 8,
            out_specs=pl.BlockSpec(memory_space=pltpu.VMEM),
            scratch_shapes=[
                pltpu.VMEM((2 * NP * GP + 1, NKT, 16, 128), BF16),
                pltpu.VMEM((D // 16, H * DH // 128, 16, 128), BF16),
                pltpu.VMEM((H * DH // 16, ND, 16, 128), BF16),
                pltpu.VMEM((D // 16, NF, 16, 128), BF16),
                pltpu.VMEM((D // 16, NF, 16, 128), BF16),
                pltpu.VMEM((FF // 16, ND, 16, 128), BF16),
                pltpu.VMEM((NP, 3, 8, 128), F32),
                pltpu.VMEM((NQ, 8, 128), F32),
                *[pltpu.VMEM((NQ + 1, 8, 128), F32)] * NB,
                *[pltpu.VMEM((2 * DH, 128), F32)] * NB,
                pltpu.VMEM((1, D), BF16),
                pltpu.SemaphoreType.DMA((5,)),
                pltpu.SemaphoreType.DMA((2,)),
            ],
            compiler_params=pltpu.CompilerParams(
                vmem_limit_bytes=124 * 1024 * 1024, flags=flags),
            name=name,
        )(A_x.reshape(1, D), _cache_tiles(A_k_cache), _cache_tiles(A_v_cache),
          _tiles(A_wq), _tiles(A_wo), _tiles(B_w1), _tiles(B_w3), _tiles(B_w2))
        return out.reshape(1, 1, D)
    return fn


pallas_interleave_layers__sliding_block_cached__glu_gated_swiglu__decode_kernel = build(lag_m=19)
```

```python
import functools
import itertools

import jax
import jax.numpy as jnp
import numpy as np
from jax import lax
import jax.experimental.pallas as pl
import jax.experimental.pallas.tpu as pltpu

F32, BF16, U32 = jnp.float32, jnp.bfloat16, jnp.uint32

D = 640
H = 32
DH = 192
SK = 32768
W = min(4096, max(256, SK // 4))
FF = 1536
NP = H // 2
NKT = W // 128
NQ = NKT // 4
ND = D // 128
NF = FF // 128
GP = 2 * DH // 16
NB = 3
AHEAD = 3
EXP2_SCALE = float(DH ** -0.5 * np.log2(np.e))
EPS = 1e-5


def _mm(a, b):
    return lax.dot_general(a, b, (((1,), (0,)), ((), ())),
                           precision=lax.Precision.DEFAULT,
                           preferred_element_type=F32)


def _rnd(a):
    return a.astype(BF16).astype(F32)


def _tile(ref, g0, c):
    return pltpu.bitcast(ref[pl.ds(g0, 8), c].reshape(64, 128), BF16)


def _allsum_rows(a):
    a = a + pltpu.roll(a, 4, 0)
    a = a + pltpu.roll(a, 2, 0)
    return a + pltpu.roll(a, 1, 0)


def _lane_sum(tiles):
    s = jnp.sum(functools.reduce(jnp.add, tiles), axis=1, keepdims=True)
    return jnp.broadcast_to(s, (8, 128))


def _ln_coef(x, even):
    m = _lane_sum(x) * (1.0 / D)
    v = _lane_sum([(t - m) * (t - m) for t in x]) * (1.0 / D)
    return jnp.where(even, 1.0, -m), lax.rsqrt(v + EPS)


def _ln_apply(t, coef):
    t = t * coef
    return t + pltpu.roll(t, 1, 0)


def _run(*gens):
    for g in gens:
        for _ in g:
            pass


def _interleave(a, b, ratio, every, fence):
    end = object()
    ta = tb = 0.0
    nxt = every
    while a is not None or b is not None:
        if a is not None and b is not None and tb >= nxt:
            fence()
            nxt = tb + every
        if b is None or (a is not None and ta * ratio <= tb):
            c = next(a, end)
            if c is end:
                a = None
            else:
                ta += c
        else:
            c = next(b, end)
            if c is end:
                b = None
            else:
                tb += c


def make_kernel(mxc_last=20, dma=True, layers=2, ratio=0.95, gblk=2, every=128,
                lag_v=0, tie=2, lag_f=36, lag_m=19, smw=20, offset=0, ratio_last=0.85, cv=1.5, nq0=3, ncs=(6, 6, 6), fskip=0):

    def kernel(x_hbm, k_hbm, v_hbm, wq_hbm, wo_hbm, w1_hbm, w3_hbm, w2_hbm, o_ref,
               kvb, wqb, wob, w1b, w3b, w2b, qs, qf, ss, *rest):
        ps, accs, (xb, sem_kv, sem_w) = rest[:NB], rest[NB:2 * NB], rest[2 * NB:]
        kvr = pltpu.annotate(kvb, no_hazard=True).bitcast(U32)
        wqr, wor = wqb.bitcast(U32), wob.bitcast(U32)
        w1r, w3r, w2r = w1b.bitcast(U32), w3b.bitcast(U32), w2b.bitcast(U32)

        def kv_copies(which, i, slot):
            src = (k_hbm, v_hbm)[which]
            return [pltpu.make_async_copy(
                src.at[pl.ds(i * GP, GP), half, pl.ds((SK - W) // 128, NKT)],
                kvb.at[pl.ds((which * NP + i) * GP, GP), :, pl.ds(half * 8, 8)],
                sem_kv.at[slot]) for half in range(2)]

        def step_copies(i):
            slot = i & 3
            return kv_copies(0, i + 1, slot) + kv_copies(1, i, slot)

        def w_copies(j, slot):
            src, dst = ((wq_hbm, wqb), (wo_hbm, wob), (w1_hbm, w1b), (w3_hbm, w3b))[j]
            return [pltpu.make_async_copy(
                src.at[:, half], dst.at[:, :, pl.ds(half * 8, 8)], sem_w.at[slot])
                for half in range(2)]

        first_copies = lambda: w_copies(0, 0) + kv_copies(0, 0, 4) + w_copies(1, 0)
        last_copies = lambda: kv_copies(1, NP - 1, 4)
        up_copies = lambda: w_copies(2, 1) + w_copies(3, 1)

        def down_copies(c):
            return [pltpu.make_async_copy(
                w2_hbm.at[:, half, c], w2b.at[:, c, pl.ds(half * 8, 8)], sem_w.at[2 + c])
                for half in range(2)]

        def start(cps):
            if dma:
                for c in cps:
                    c.start()

        def wait(cps):
            if dma:
                for c in cps:
                    c.wait()

        x_copy = pltpu.make_async_copy(x_hbm, xb, sem_w.at[1])
        x_copy.start()
        start(first_copies())
        for i in range(AHEAD):
            start(step_copies(i))
        x_copy.wait()
        x = jnp.broadcast_to(xb[...].astype(F32), (8, D))
        x = [x[:, c * 128:(c + 1) * 128] for c in range(ND)]

        row = lax.broadcasted_iota(jnp.int32, (8, 128), 0)
        lane = lax.broadcasted_iota(jnp.int32, (8, 128), 1)
        head_of_lane = [jnp.zeros_like(lane), (lane >= 64).astype(jnp.int32),
                        jnp.ones_like(lane)]
        head_mask = [(row & 1) == h for h in head_of_lane]
        slot_mask = [(row >> 1) == s for s in range(4)]

        even = (row & 1) == 0

        def with_ones(x):
            return [jnp.where(even, t, 1.0) for t in x]

        spot = jnp.max(pltpu.bitcast(x[0], jnp.int32) & 1)
        never = lane == spot + 128
        hist = {}

        def reset():
            hist.update(vpu=[], mxu=[], due=[], n=0)

        def fence():
            if len(hist["mxu"]) > lag_m:
                kvr[2 * NP * GP, spot] = pltpu.bitcast(hist["mxu"][-1 - lag_m], U32)

        def tied(a):
            hist["n"] += 1
            if hist["due"] and hist["due"][0][0] <= hist["n"]:
                return jnp.where(never, hist["due"].pop(0)[1], a)
            if hist["n"] % tie == 0 and len(hist["vpu"]) > lag_v:
                live = hist["vpu"][-1 - lag_v]
                return jnp.where(never, live[(hist["n"] // tie) % len(live)], a)
            return a

        def mm(a, b, mask=None):
            a = tied(a)
            t = _mm(a if mask is None else jnp.where(mask, a, 0.0), b)
            hist["mxu"].append(t)
            return t

        def matvec(a, ref, g0, cols, out):
            for n, c in enumerate(cols):
                for kt, at in enumerate(a):
                    t = mm(at, _tile(ref, g0 + kt * 8, c))
                    out[n] = t if out[n] is None else out[n] + t
                    yield 8

        def q_partial(xo, kt, i):
            q = [None] * 3 if kt == 0 else [qs[i, dt] for dt in range(3)]
            yield from matvec(xo, wqr, kt * 8, [i * 3 + dt for dt in range(3)], q)
            for dt in range(3):
                qs[i, dt] = q[dt]

        def q_finish(xo, coef, i):
            q = [qs[i, dt] for dt in range(3)]
            yield from matvec(xo, wqr, (ND - 1) * 8, [i * 3 + dt for dt in range(3)], q)
            for dt in range(3):
                qf[i, dt] = jnp.where(head_mask[dt], _rnd(_ln_apply(q[dt], coef)), 0.0)

        def scores(i, buf, scale, meanwhile=()):
            q = [qf[i, dt] for dt in range(3)]
            m = None
            for j in range(NQ):
                s = None
                for sl in range(4):
                    for dt in range(3):
                        t = mm(q[dt], _tile(kvr, i * GP + dt * 8, 4 * j + sl), slot_mask[sl])
                        s = t if s is None else s + t
                        yield 8
                ss[j] = s
                m = s if m is None else jnp.maximum(m, s)
            m = jnp.broadcast_to(jnp.max(m, axis=1, keepdims=True), (8, 128))
            m = jnp.maximum(m, pltpu.roll(m, 4, 0))
            m = jnp.maximum(m, pltpu.roll(m, 2, 0))
            yield from meanwhile
            l = None
            for j in range(NQ):
                p = jnp.exp2((ss[j] - m) * scale)
                ps[buf][j] = p
                l = p if l is None else l + p
            ps[buf][NQ] = l

        def transpose_v(i, nc):
            def body(c, carry):
                for dt in range(3):
                    g0 = (NP + i) * GP + dt * 8
                    t = pltpu.bitcast(_tile(kvr, g0, c).T, U32)
                    kvr[pl.ds(g0, 8), c] = t.reshape(8, 8, 128)
                return carry
            lax.fori_loop(NKT - nc, NKT, body, 0)

        def pv_vpu(i, buf, nc, side=iter(())):
            for hh in range(2):
                for gb in range(0, 12, gblk):
                    yield next(side, 0) if (hh * 12 + gb) // gblk >= fskip else 0
                    lo = [None] * gblk
                    hi = [None] * gblk
                    for c in range(NKT - nc):
                        p = ps[buf][c // 4, pl.ds((c % 4) * 2 + hh, 8, stride=0), :]
                        for g in range(gblk):
                            w = kvr[(NP + i) * GP + hh * 12 + gb + g, c]
                            a = pltpu.bitcast(w << 16, F32) * p
                            b = pltpu.bitcast(w & np.uint32(0xFFFF0000), F32) * p
                            lo[g] = a if lo[g] is None else lo[g] + a
                            hi[g] = b if hi[g] is None else hi[g] + b
                            yield cv
                        hist["vpu"].append(lo + hi)
                    for g in range(gblk):
                        r0 = (hh * 12 + gb + g) * 16
                        accs[buf][pl.ds(r0, 8, stride=2), :] = lo[g]
                        accs[buf][pl.ds(r0 + 1, 8, stride=2), :] = hi[g]

        def pv_mxu(i, buf, nc, om):
            for c in range(NKT - nc, NKT):
                p = _rnd(ps[buf][c // 4])
                for dt in range(3):
                    t = mm(p, _tile(kvr, (NP + i) * GP + dt * 8, c), slot_mask[c % 4])
                    om[dt] = t if om[dt] is None else om[dt] + t
                    yield 8

        def pv_finish(buf, om, o):
            l = _lane_sum([ps[buf][NQ]])
            l = l + pltpu.roll(l, 4, 0)
            l = l + pltpu.roll(l, 2, 0)
            inv = 1.0 / l
            inv_other = pltpu.roll(inv, 1, 0)
            for dt in range(3):
                t = accs[buf][pl.ds(dt * 128, 128), :].T.reshape(16, 8, 128)
                t = jnp.sum(t, axis=0) + jnp.where(head_mask[dt], om[dt], 0.0)
                t = _allsum_rows(t)
                o[dt] = _rnd(t * jnp.where(head_mask[dt], inv, inv_other))
                hist["due"].append((hist["n"] + lag_f, o[dt]))
                yield 8

        def out_proj(o, i, y):
            return matvec(o, wor, i * GP, range(ND), y)

        def attention_streaming(x):
            wait(first_copies())
            xo, (coef, r) = with_ones(x), _ln_coef(x, even)
            scale = r * EXP2_SCALE
            lax.fori_loop(0, NP, lambda i, c: _run(
                q_partial(xo[:-1], 0, i), q_finish(xo[-1:], coef, i)), None)
            reset()
            _run(scores(0, 0, scale))

            def attend(i, nc, y):
                reset()
                transpose_v(i, nc)
                om, o, y = [None] * 3, [None] * 3, list(y)
                _run(pv_mxu(i, 0, nc, om), pv_vpu(i, 0, nc), pv_finish(0, om, o))
                reset()
                _run(out_proj(o, i, y))
                return y

            def step(i, nc, y):
                @pl.when(i + AHEAD < NP - 1)
                def _():
                    start(step_copies(i + AHEAD))

                @pl.when(i + AHEAD == NP - 1)
                def _():
                    start(last_copies() + up_copies())
                    for c in range(ND):
                        start(down_copies(c))

                wait(step_copies(i))
                y = attend(i, nc, y)
                _run(scores(i + 1, 0, scale))
                return y

            def steps(t, y):
                for u in range(NB):
                    y = step(t * NB + u, ncs[u], y)
                return y

            zeros = [jnp.zeros((8, 128), F32)] * ND
            if len(set(ncs)) == 1:
                y = lax.fori_loop(0, NP - 1, lambda i, y: step(i, ncs[0], y), zeros)
            else:
                y = lax.fori_loop(0, (NP - 1) // NB, steps, zeros)
            wait(last_copies())
            return attend(NP - 1, mxc_last, y)

        def attention_resident(x):
            reset()
            accs[NB - 1][...] = jnp.zeros((2 * DH, 128), F32)
            ps[NB - 1][NQ] = jnp.ones((8, 128), F32)
            xo, (coef, r) = with_ones(x[-1:]), _ln_coef(x, even)
            scale = r * EXP2_SCALE
            _run(*[q_finish(xo, coef, i) for i in range(nq0)],
                 scores(0, 0, scale,
                        itertools.chain(*[q_finish(xo, coef, i) for i in range(nq0, NP)])))

            def step(t, carry):
                om_prev, y = carry
                y = list(y)
                reset()
                ma, va = [], [iter([offset])]
                for u in range(NB):
                    i = t * NB + u
                    om, o = [None] * 3, [None] * 3
                    rest = itertools.chain(
                        pv_mxu(i, u, ncs[u], om),
                        out_proj(o, jnp.maximum(i - 1, 0), y))
                    ma += [scores(i + 1, (u + 1) % NB, scale, itertools.islice(rest, smw)), rest]
                    va += [pv_vpu(i, u, ncs[u], pv_finish((u - 1) % NB, om_prev, o))]
                    om_prev = om
                _interleave(itertools.chain(*ma), itertools.chain(*va), ratio, every, fence)
                return om_prev, y

            zero = jnp.zeros((8, 128), F32)
            om_prev, y = lax.fori_loop(0, (NP - 1) // NB, step, ([zero] * 3, [zero] * ND))
            y = list(y)
            reset()
            om, o = [None] * 3, [None] * 3
            _interleave(
                itertools.chain(pv_mxu(NP - 1, 0, mxc_last, om), out_proj(o, NP - 2, y)),
                pv_vpu(NP - 1, 0, mxc_last, pv_finish(NB - 1, om_prev, o)),
                ratio_last, every, fence)
            o = [None] * 3
            _run(pv_finish(0, om, o))
            reset()
            _run(out_proj(o, NP - 1, y))
            return y

        def ffn_hidden(x):
            reset()
            xo, (coef, r) = with_ones(x), _ln_coef(x, even)
            coef = coef * r
            h = []
            for ft in range(NF):
                gate, up = [None], [None]
                _run(matvec(xo, w1r, 0, [ft], gate), matvec(xo, w3r, 0, [ft], up))
                gate, up = _ln_apply(gate[0], coef), _ln_apply(up[0], coef)
                h.append(_rnd(gate / (1.0 + jnp.exp(-gate)) * up))
            return h

        def add(x, y):
            return [_rnd(a + b) for a, b in zip(x, y)]

        def resident_layer(_, x):
            x = add(x, attention_resident(x))
            h = ffn_hidden(x)
            f = [None] * ND
            _run(*[matvec([h[kt]], w2r, kt * 8, range(ND), f) for kt in range(NF)])
            return add(x, f)

        if dma:
            reset()
            x = add(x, attention_streaming(x))
            wait(up_copies())
            h = ffn_hidden(x)
            for c in range(ND):
                wait(down_copies(c))
                f = [None]
                _run(matvec(h, w2r, 0, [c], f))
                x[c] = _rnd(x[c] + f[0])
                if c < ND - 1:
                    xo = with_ones(x[c:c + 1])
                    _run(*[q_partial(xo, c, i) for i in range(NP)])
            x = resident_layer(0, x)
        else:
            x = lax.fori_loop(0, layers, resident_layer, x)
        o_ref[...] = jnp.concatenate(x, axis=1)[0:1].astype(BF16)

    return kernel


def _tiles(a):
    r, c = a.shape
    return a.reshape(r // 16, 2, 8, c // 128, 128).transpose(0, 1, 3, 2, 4)


def _cache_tiles(a):
    a = a.reshape(H, SK // 128, 128, DH // 8, 8).transpose(0, 3, 1, 4, 2)
    return a.reshape(H * DH // 16, 2, SK // 128, 8, 128)


def build(name="fused", flags=None, **kw):
    @jax.jit
    def fn(A_x, A_k_cache, A_v_cache, A_wq, A_wo, B_x, B_w1, B_w3, B_w2):
        del B_x
        hbm = pl.BlockSpec(memory_space=pl.ANY)
        out = pl.pallas_call(
            make_kernel(**kw),
            out_shape=jax.ShapeDtypeStruct((1, D), BF16),
            in_specs=[hbm] * 8,
            out_specs=pl.BlockSpec(memory_space=pltpu.VMEM),
            scratch_shapes=[
                pltpu.VMEM((2 * NP * GP + 1, NKT, 16, 128), BF16),
                pltpu.VMEM((D // 16, H * DH // 128, 16, 128), BF16),
                pltpu.VMEM((H * DH // 16, ND, 16, 128), BF16),
                pltpu.VMEM((D // 16, NF, 16, 128), BF16),
                pltpu.VMEM((D // 16, NF, 16, 128), BF16),
                pltpu.VMEM((FF // 16, ND, 16, 128), BF16),
                pltpu.VMEM((NP, 3, 8, 128), F32),
                pltpu.VMEM((NP, 3, 8, 128), F32),
                pltpu.VMEM((NQ, 8, 128), F32),
                *[pltpu.VMEM((NQ + 1, 8, 128), F32)] * NB,
                *[pltpu.VMEM((2 * DH, 128), F32)] * NB,
                pltpu.VMEM((1, D), BF16),
                pltpu.SemaphoreType.DMA((5,)),
                pltpu.SemaphoreType.DMA((2 + ND,)),
            ],
            compiler_params=pltpu.CompilerParams(
                vmem_limit_bytes=124 * 1024 * 1024, flags=flags),
            name=name,
        )(A_x.reshape(1, D), _cache_tiles(A_k_cache), _cache_tiles(A_v_cache),
          _tiles(A_wq), _tiles(A_wo), _tiles(B_w1), _tiles(B_w3), _tiles(B_w2))
        return out.reshape(1, 1, D)
    return fn


pallas_interleave_layers__sliding_block_cached__glu_gated_swiglu__decode_kernel = build(ratio=0.93)
```

```python
import functools
import itertools

import jax
import jax.numpy as jnp
import numpy as np
from jax import lax
import jax.experimental.pallas as pl
import jax.experimental.pallas.tpu as pltpu

F32, BF16, U32 = jnp.float32, jnp.bfloat16, jnp.uint32

D = 640
H = 32
DH = 192
SK = 32768
W = min(4096, max(256, SK // 4))
FF = 1536
NP = H // 2
NKT = W // 128
NQ = NKT // 4
ND = D // 128
NF = FF // 128
GP = 2 * DH // 16
NB = 3
AHEAD = 3
EXP2_SCALE = float(DH ** -0.5 * np.log2(np.e))
EPS = 1e-5
SCALE, OUT = 0, 1


def _mm(a, b):
    return lax.dot_general(a, b, (((1,), (0,)), ((), ())),
                           precision=lax.Precision.DEFAULT,
                           preferred_element_type=F32)


def _rnd(a):
    return a.astype(BF16).astype(F32)


def _tile(ref, g0, c):
    return pltpu.bitcast(ref[pl.ds(g0, 8), c].reshape(64, 128), BF16)


def _allsum_rows(a):
    a = a + pltpu.roll(a, 4, 0)
    a = a + pltpu.roll(a, 2, 0)
    return a + pltpu.roll(a, 1, 0)


def _lane_sum(tiles):
    s = jnp.sum(functools.reduce(jnp.add, tiles), axis=1, keepdims=True)
    return jnp.broadcast_to(s, (8, 128))


def _ln_coef(x, even):
    m = _lane_sum(x) * (1.0 / D)
    v = _lane_sum([(t - m) * (t - m) for t in x]) * (1.0 / D)
    return jnp.where(even, 1.0, -m), lax.rsqrt(v + EPS)


def _ln_apply(t, coef):
    t = t * coef
    return t + pltpu.roll(t, 1, 0)


def _run(*gens):
    for g in gens:
        for _ in g:
            pass


def _interleave(a, b, ratio, every, fence):
    end = object()
    ta = tb = 0.0
    nxt = every
    while a is not None or b is not None:
        if a is not None and b is not None and tb >= nxt:
            fence()
            nxt = tb + every
        if b is None or (a is not None and ta * ratio <= tb):
            c = next(a, end)
            if c is end:
                a = None
            else:
                ta += c
        else:
            c = next(b, end)
            if c is end:
                b = None
            else:
                tb += c


def make_kernel(mxc_last=20, dma=True, layers=2, ratio=0.93, gblk=2, every=128,
                lag_v=0, tie=2, lag_f=36, lag_m=19, smw=20, offset=0, ratio_last=0.85, cv=1.5, nq0=3, mxc=6, kcuts=(0, 8, 12, 15, 16), fskip=0, nohaz=False):

    def kernel(x_hbm, k_hbm, v_hbm, wq_hbm, wo_hbm, w1_hbm, w3_hbm, w2_hbm, o_ref,
               kvb, wqb, wob, w1b, w3b, w2b, qs, qf, ss, ys, misc, *rest):
        ps, pb, accs, (xb, sems) = rest[:NB], rest[NB:2 * NB], rest[2 * NB:3 * NB], rest[3 * NB:]
        kvr = (pltpu.annotate(kvb, no_hazard=True) if nohaz else kvb).bitcast(U32)
        wqr, wor = wqb.bitcast(U32), wob.bitcast(U32)
        w1r, w3r, w2r = w1b.bitcast(U32), w3b.bitcast(U32), w2b.bitcast(U32)

        def kv_copies(which, i, n, slot):
            src = (k_hbm, v_hbm)[which]
            return [pltpu.make_async_copy(
                src.at[pl.ds(i * GP, n * GP), half, pl.ds((SK - W) // 128, NKT)],
                kvb.at[pl.ds((which * NP + i) * GP, n * GP), :, pl.ds(half * 8, 8)],
                sems.at[slot]) for half in range(2)]

        def w_copies(src, dst, slot, c=slice(None)):
            return [pltpu.make_async_copy(
                src.at[:, half, c], dst.at[:, c, pl.ds(half * 8, 8)], sems.at[slot])
                for half in range(2)]

        x_copies = [pltpu.make_async_copy(x_hbm, xb, sems.at[0])]
        first_copies = w_copies(wq_hbm, wqb, 1) + kv_copies(1, 0, NP, 1)
        wo_copies = w_copies(wo_hbm, wob, 2)
        k_copies = [kv_copies(0, a, b - a, 3 + n)
                    for n, (a, b) in enumerate(zip(kcuts, kcuts[1:]))]
        ns = 3 + len(k_copies)
        w1_copies, w3_copies = w_copies(w1_hbm, w1b, ns), w_copies(w3_hbm, w3b, ns + 1)
        w2_copies = [w_copies(w2_hbm, w2b, ns + 2 + c, c) for c in range(ND)]

        def start(cps):
            if dma:
                for c in cps:
                    c.start()

        def wait(cps):
            if dma:
                for c in cps:
                    c.wait()

        x_copies[0].start()
        for cps in (first_copies, wo_copies, *k_copies, w1_copies, w3_copies, *w2_copies):
            start(cps)
        x_copies[0].wait()
        x = jnp.broadcast_to(xb[...].astype(F32), (8, D))
        x = [x[:, c * 128:(c + 1) * 128] for c in range(ND)]

        row = lax.broadcasted_iota(jnp.int32, (8, 128), 0)
        lane = lax.broadcasted_iota(jnp.int32, (8, 128), 1)
        head_of_lane = [jnp.zeros_like(lane), (lane >= 64).astype(jnp.int32),
                        jnp.ones_like(lane)]
        head_mask = [(row & 1) == h for h in head_of_lane]
        slot_mask = [(row >> 1) == s for s in range(4)]

        even = (row & 1) == 0

        def with_ones(x):
            return [jnp.where(even, t, 1.0) for t in x]

        spot = jnp.max(pltpu.bitcast(x[0], jnp.int32) & 1)
        never = lane == spot + 128
        hist = {}

        def reset():
            hist.update(vpu=[], mxu=[], due=[], n=0)

        def fence():
            if len(hist["mxu"]) > lag_m:
                kvr[2 * NP * GP, spot] = pltpu.bitcast(hist["mxu"][-1 - lag_m], U32)

        def tied(a):
            hist["n"] += 1
            if hist["due"] and hist["due"][0][0] <= hist["n"]:
                return jnp.where(never, hist["due"].pop(0)[1], a)
            if hist["n"] % tie == 0 and len(hist["vpu"]) > lag_v:
                live = hist["vpu"][-1 - lag_v]
                return jnp.where(never, live[(hist["n"] // tie) % len(live)], a)
            return a

        def mm(a, b, mask=None):
            a = tied(a)
            t = _mm(a if mask is None else jnp.where(mask, a, 0.0), b)
            hist["mxu"].append(t)
            return t

        def matvec(a, ref, g0, cols, out):
            for n, c in enumerate(cols):
                for kt, at in enumerate(a):
                    t = mm(at, _tile(ref, g0 + kt * 8, c))
                    out[n] = t if out[n] is None else out[n] + t
                    yield 8

        def q_partial(xo, kt, i):
            q = [None] * 3 if kt == 0 else [qs[i, dt] for dt in range(3)]
            yield from matvec(xo, wqr, kt * 8, [i * 3 + dt for dt in range(3)], q)
            for dt in range(3):
                qs[i, dt] = q[dt]

        def q_finish(xo, coef, i):
            q = [qs[i, dt] for dt in range(3)]
            yield from matvec(xo, wqr, (ND - 1) * 8, [i * 3 + dt for dt in range(3)], q)
            for dt in range(3):
                qf[i, dt] = jnp.where(head_mask[dt], _rnd(_ln_apply(q[dt], coef)), 0.0)

        def scores(i, buf, nc, meanwhile=()):
            q = [qf[i, dt] for dt in range(3)]
            m = None
            for j in range(NQ):
                s = None
                for sl in range(4):
                    for dt in range(3):
                        t = mm(q[dt], _tile(kvr, i * GP + dt * 8, 4 * j + sl), slot_mask[sl])
                        s = t if s is None else s + t
                        yield 8
                ss[j] = s
                m = s if m is None else jnp.maximum(m, s)
            m = jnp.broadcast_to(jnp.max(m, axis=1, keepdims=True), (8, 128))
            m = jnp.maximum(m, pltpu.roll(m, 4, 0))
            m = jnp.maximum(m, pltpu.roll(m, 2, 0))
            yield from meanwhile
            l = None
            for j in range(NQ):
                p = jnp.exp2((ss[j] - m) * misc[SCALE])
                ps[buf][j] = p
                for c in range(4 * j, min(4 * j + 4, NKT - nc)):
                    for hh in range(2):
                        r = (c % 4) * 2 + hh
                        pb[buf][pl.ds(c * 16 + hh, 8, stride=2), :] = jnp.broadcast_to(p[r:r + 1], (8, 128))
                l = p if l is None else l + p
            ps[buf][NQ] = l

        def transpose_v(i, nc):
            def body(c, carry):
                for dt in range(3):
                    g0 = (NP + i) * GP + dt * 8
                    t = pltpu.bitcast(_tile(kvr, g0, c).T, U32)
                    kvr[pl.ds(g0, 8), c] = t.reshape(8, 8, 128)
                return carry
            lax.fori_loop(NKT - nc, NKT, body, 0)

        def pv_vpu(i, buf, nc, side=iter(())):
            for hh in range(2):
                for gb in range(0, 12, gblk):
                    yield next(side, 0) if (hh * 12 + gb) // gblk >= fskip else 0
                    lo = [None] * gblk
                    hi = [None] * gblk
                    for c in range(NKT - nc):
                        p = pb[buf][pl.ds(c * 16 + hh, 8, stride=2), :]
                        for g in range(gblk):
                            w = kvr[(NP + i) * GP + hh * 12 + gb + g, c]
                            a = pltpu.bitcast(w << 16, F32) * p
                            b = pltpu.bitcast(w & np.uint32(0xFFFF0000), F32) * p
                            lo[g] = a if lo[g] is None else lo[g] + a
                            hi[g] = b if hi[g] is None else hi[g] + b
                            yield cv
                        hist["vpu"].append(lo + hi)
                    for g in range(gblk):
                        r0 = (hh * 12 + gb + g) * 16
                        accs[buf][pl.ds(r0, 8, stride=2), :] = lo[g]
                        accs[buf][pl.ds(r0 + 1, 8, stride=2), :] = hi[g]

        def pv_mxu(i, buf, nc):
            om = [None] * 3
            for c in range(NKT - nc, NKT):
                p = _rnd(ps[buf][c // 4])
                for dt in range(3):
                    t = mm(p, _tile(kvr, (NP + i) * GP + dt * 8, c), slot_mask[c % 4])
                    om[dt] = t if om[dt] is None else om[dt] + t
                    yield 8
            for dt in range(3):
                ps[buf][NQ + 1 + dt] = om[dt]

        def pv_finish(buf):
            l = _lane_sum([ps[buf][NQ]])
            l = l + pltpu.roll(l, 4, 0)
            l = l + pltpu.roll(l, 2, 0)
            inv = 1.0 / l
            inv_other = pltpu.roll(inv, 1, 0)
            for dt in range(3):
                t = accs[buf][pl.ds(dt * 128, 128), :].T.reshape(16, 8, 128)
                t = jnp.sum(t, axis=0) + jnp.where(head_mask[dt], ps[buf][NQ + 1 + dt], 0.0)
                t = _allsum_rows(t)
                o = _rnd(t * jnp.where(head_mask[dt], inv, inv_other))
                misc[OUT + dt] = o
                hist["due"].append((hist["n"] + lag_f, o))
                yield 8

        def out_proj(i):
            o = [misc[OUT + dt] for dt in range(3)]
            for c in range(ND):
                y = [ys[c]]
                yield from matvec(o, wor, i * GP, [c], y)
                ys[c] = y[0]

        def attention_streaming(x):
            wait(first_copies)
            xo, (coef, r) = with_ones(x), _ln_coef(x, even)
            misc[SCALE] = r * EXP2_SCALE

            def prepare(i, carry):
                _run(q_partial(xo[:-1], 0, i), q_finish(xo[-1:], coef, i))
                transpose_v(i, jnp.where(i == NP - 1, mxc_last, mxc))
                return carry

            lax.fori_loop(0, NP, prepare, 0)
            wait(wo_copies)

            ys[...] = jnp.zeros(ys.shape, F32)

            def attend(i, nc):
                reset()
                _run(scores(i, 0, nc), pv_mxu(i, 0, nc), pv_vpu(i, 0, nc), pv_finish(0))
                reset()
                _run(out_proj(i))

            def step(i, carry):
                for first, cps in zip(kcuts, k_copies[:-1]):
                    pl.when(i == first)(functools.partial(wait, cps))
                attend(i, mxc)
                return carry

            lax.fori_loop(0, NP - 1, step, 0)
            wait(k_copies[-1])
            attend(NP - 1, mxc_last)
            return [ys[c] for c in range(ND)]

        def attention_resident(x):
            reset()
            accs[NB - 1][pl.ds(0, 2 * DH), :] = jnp.zeros((2 * DH, 128), F32)
            ps[NB - 1][NQ] = jnp.ones((8, 128), F32)
            ps[NB - 1][pl.ds(NQ + 1, 3)] = jnp.zeros((3, 8, 128), F32)
            ys[...] = jnp.zeros(ys.shape, F32)
            xo, (coef, r) = with_ones(x[-1:]), _ln_coef(x, even)
            misc[SCALE] = r * EXP2_SCALE
            _run(*[q_finish(xo, coef, i) for i in range(nq0)],
                 scores(0, 0, mxc,
                        itertools.chain(*[q_finish(xo, coef, i) for i in range(nq0, NP)])))

            def step(t, carry):
                reset()
                ma, va = [], [iter([offset])]
                for u in range(NB):
                    i = t * NB + u
                    rest = itertools.chain(pv_mxu(i, u, mxc), out_proj(jnp.maximum(i - 1, 0)))
                    ma += [scores(i + 1, (u + 1) % NB, mxc, itertools.islice(rest, smw)), rest]
                    va += [pv_vpu(i, u, mxc, pv_finish((u - 1) % NB))]
                _interleave(itertools.chain(*ma), itertools.chain(*va), ratio, every, fence)
                return carry

            lax.fori_loop(0, (NP - 1) // NB, step, 0)
            reset()
            _interleave(
                itertools.chain(pv_mxu(NP - 1, 0, mxc_last), out_proj(NP - 2)),
                pv_vpu(NP - 1, 0, mxc_last, pv_finish(NB - 1)),
                ratio_last, every, fence)
            _run(pv_finish(0))
            reset()
            _run(out_proj(NP - 1))
            return [ys[c] for c in range(ND)]

        def ffn_hidden(x, first):
            reset()
            xo, (coef, r) = with_ones(x), _ln_coef(x, even)
            coef = coef * r
            gate, up, h = [None] * NF, [None] * NF, []
            if first:
                wait(w1_copies)
                _run(matvec(xo, w1r, 0, range(NF), gate))
                wait(w3_copies)
                _run(matvec(xo, w3r, 0, range(NF), up))
            for ft in range(NF):
                g, u = gate[ft:ft + 1], up[ft:ft + 1]
                if not first:
                    _run(matvec(xo, w1r, 0, [ft], g), matvec(xo, w3r, 0, [ft], u))
                g, u = _ln_apply(g[0], coef), _ln_apply(u[0], coef)
                h.append(_rnd(g / (1.0 + jnp.exp(-g)) * u))
            return h

        def add(x, y):
            return [_rnd(a + b) for a, b in zip(x, y)]

        def resident_layer(_, x):
            x = add(x, attention_resident(x))
            h = ffn_hidden(x, False)
            f = [None] * ND
            _run(*[matvec([h[kt]], w2r, kt * 8, range(ND), f) for kt in range(NF)])
            return add(x, f)

        if dma:
            reset()
            x = add(x, attention_streaming(x))
            h = ffn_hidden(x, True)
            for c in range(ND):
                wait(w2_copies[c])
                f = [None]
                _run(matvec(h, w2r, 0, [c], f))
                x[c] = _rnd(x[c] + f[0])
                if c < ND - 1:
                    xo = with_ones(x[c:c + 1])
                    _run(*[q_partial(xo, c, i) for i in range(NP)])
            x = resident_layer(0, x)
        else:
            x = lax.fori_loop(0, layers, resident_layer, x)
        o_ref[...] = jnp.concatenate(x, axis=1)[0:1].astype(BF16)

    return kernel


def _tiles(a):
    r, c = a.shape
    return a.reshape(r // 16, 2, 8, c // 128, 128).transpose(0, 1, 3, 2, 4)


def _cache_tiles(a):
    a = a.reshape(H, SK // 128, 128, DH // 8, 8).transpose(0, 3, 1, 4, 2)
    return a.reshape(H * DH // 16, 2, SK // 128, 8, 128)


def build(name="fused", flags=None, **kw):
    @jax.jit
    def fn(A_x, A_k_cache, A_v_cache, A_wq, A_wo, B_x, B_w1, B_w3, B_w2):
        del B_x
        hbm = pl.BlockSpec(memory_space=pl.ANY)
        out = pl.pallas_call(
            make_kernel(**kw),
            out_shape=jax.ShapeDtypeStruct((1, D), BF16),
            in_specs=[hbm] * 8,
            out_specs=pl.BlockSpec(memory_space=pltpu.VMEM),
            scratch_shapes=[
                pltpu.VMEM((2 * NP * GP + 1, NKT, 16, 128), BF16),
                pltpu.VMEM((D // 16, H * DH // 128, 16, 128), BF16),
                pltpu.VMEM((H * DH // 16, ND, 16, 128), BF16),
                pltpu.VMEM((D // 16, NF, 16, 128), BF16),
                pltpu.VMEM((D // 16, NF, 16, 128), BF16),
                pltpu.VMEM((FF // 16, ND, 16, 128), BF16),
                pltpu.VMEM((NP, 3, 8, 128), F32),
                pltpu.VMEM((NP, 3, 8, 128), F32),
                pltpu.VMEM((NQ, 8, 128), F32),
                pltpu.VMEM((ND, 8, 128), F32),
                pltpu.VMEM((4, 8, 128), F32),
                *[pltpu.VMEM((NQ + 4, 8, 128), F32)] * NB,
                *[pltpu.VMEM((NKT * 16, 128), F32)] * NB,
                *[pltpu.VMEM((2 * DH + 8, 128), F32)] * NB,
                pltpu.VMEM((1, D), BF16),
                pltpu.SemaphoreType.DMA((14,)),
            ],
            compiler_params=pltpu.CompilerParams(
                vmem_limit_bytes=124 * 1024 * 1024, flags=flags),
            name=name,
        )(A_x.reshape(1, D), _cache_tiles(A_k_cache), _cache_tiles(A_v_cache),
          _tiles(A_wq), _tiles(A_wo), _tiles(B_w1), _tiles(B_w3), _tiles(B_w2))
        return out.reshape(1, 1, D)
    return fn


pallas_interleave_layers__sliding_block_cached__glu_gated_swiglu__decode_kernel = build()
```

```python
import functools
import itertools

import jax
import jax.numpy as jnp
import numpy as np
from jax import lax
import jax.experimental.pallas as pl
import jax.experimental.pallas.tpu as pltpu

F32, BF16, U32 = jnp.float32, jnp.bfloat16, jnp.uint32

D = 640
H = 32
DH = 192
SK = 32768
W = min(4096, max(256, SK // 4))
FF = 1536
EPS = 1e-5
EXP2_SCALE = float(DH ** -0.5 * np.log2(np.e))

NP = H // 2
GP = 2 * DH // 16
NKT = W // 128
NQ = NKT // 4
ND = D // 128
NF = FF // 128

NB = 3
MXU_TILES = 6
MXU_TILES_LAST = 20
K_CUTS = (0, 8, 12, 15, NP)
SCALE, OUT = 0, 1

RATIO, RATIO_LAST = 0.93, 1.0
FENCE_EVERY, FENCE_LAG = 128, 19
TIE_EVERY, FINISH_LAG, SOFTMAX_LAG = 2, 36, 20


def _mm(a, b):
    return lax.dot_general(a, b, (((1,), (0,)), ((), ())),
                           precision=lax.Precision.DEFAULT,
                           preferred_element_type=F32)


def _rnd(a):
    return a.astype(BF16).astype(F32)


def _tile(ref, g0, c):
    return pltpu.bitcast(ref[pl.ds(g0, 8), c].reshape(64, 128), BF16)


def _allsum_rows(a):
    a = a + pltpu.roll(a, 4, 0)
    a = a + pltpu.roll(a, 2, 0)
    return a + pltpu.roll(a, 1, 0)


def _lane_sum(tiles):
    s = jnp.sum(functools.reduce(jnp.add, tiles), axis=1, keepdims=True)
    return jnp.broadcast_to(s, (8, 128))


def _ln_stats(x, even):
    m = _lane_sum(x) * (1.0 / D)
    v = _lane_sum([(t - m) * (t - m) for t in x]) * (1.0 / D)
    return jnp.where(even, 1.0, -m), lax.rsqrt(v + EPS)


def _ln_apply(t, coef):
    t = t * coef
    return t + pltpu.roll(t, 1, 0)


def _run(*gens):
    for g in gens:
        for _ in g:
            pass


def _interleave(a, b, ratio, fence):
    end = object()
    ta = tb = 0.0
    nxt = FENCE_EVERY
    while a is not None or b is not None:
        if a is not None and b is not None and tb >= nxt:
            fence()
            nxt = tb + FENCE_EVERY
        if b is None or (a is not None and ta * ratio <= tb):
            c = next(a, end)
            if c is end:
                a = None
            else:
                ta += c
        else:
            c = next(b, end)
            if c is end:
                b = None
            else:
                tb += c


def _kernel(x_hbm, k_hbm, v_hbm, wq_hbm, wo_hbm, w1_hbm, w3_hbm, w2_hbm, o_ref,
            kvb, wqb, wob, w1b, w3b, w2b, qs, qf, ss, ys, misc, *rest):
    ps, pb, accs = rest[:NB], rest[NB:2 * NB], rest[2 * NB:3 * NB]
    xb, sems = rest[3 * NB:]
    kvr, wqr, wor = kvb.bitcast(U32), wqb.bitcast(U32), wob.bitcast(U32)
    w1r, w3r, w2r = w1b.bitcast(U32), w3b.bitcast(U32), w2b.bitcast(U32)

    def kv_copies(which, i, n, slot):
        src = (k_hbm, v_hbm)[which]
        return [pltpu.make_async_copy(
            src.at[pl.ds(i * GP, n * GP), half, pl.ds((SK - W) // 128, NKT)],
            kvb.at[pl.ds((which * NP + i) * GP, n * GP), :, pl.ds(half * 8, 8)],
            sems.at[slot]) for half in range(2)]

    def w_copies(src, dst, slot, c=slice(None)):
        return [pltpu.make_async_copy(
            src.at[:, half, c], dst.at[:, c, pl.ds(half * 8, 8)], sems.at[slot])
            for half in range(2)]

    def wait(copies):
        for c in copies:
            c.wait()

    x_copies = [pltpu.make_async_copy(x_hbm, xb, sems.at[0])]
    first_copies = w_copies(wq_hbm, wqb, 1) + kv_copies(1, 0, NP, 1)
    wo_copies = w_copies(wo_hbm, wob, 2)
    k_copies = [kv_copies(0, a, b - a, 3 + n)
                for n, (a, b) in enumerate(zip(K_CUTS, K_CUTS[1:]))]
    ns = 3 + len(k_copies)
    w1_copies, w3_copies = w_copies(w1_hbm, w1b, ns), w_copies(w3_hbm, w3b, ns + 1)
    w2_copies = [w_copies(w2_hbm, w2b, ns + 2 + c, c) for c in range(ND)]
    for c in itertools.chain(x_copies, first_copies, wo_copies, *k_copies,
                             w1_copies, w3_copies, *w2_copies):
        c.start()

    wait(x_copies)
    x = jnp.broadcast_to(xb[...].astype(F32), (8, D))
    x = [x[:, c * 128:(c + 1) * 128] for c in range(ND)]

    row = lax.broadcasted_iota(jnp.int32, (8, 128), 0)
    lane = lax.broadcasted_iota(jnp.int32, (8, 128), 1)
    head_of_lane = [jnp.zeros_like(lane), (lane >= 64).astype(jnp.int32),
                    jnp.ones_like(lane)]
    head_mask = [(row & 1) == h for h in head_of_lane]
    slot_mask = [(row >> 1) == s for s in range(4)]
    even = (row & 1) == 0

    def with_ones(x):
        return [jnp.where(even, t, 1.0) for t in x]

    spot = jnp.max(pltpu.bitcast(x[0], jnp.int32) & 1)
    never = lane == spot + 128
    hist = {}

    def reset():
        hist.update(vpu=[], mxu=[], due=[], n=0)

    def fence():
        if len(hist["mxu"]) > FENCE_LAG:
            kvr[2 * NP * GP, spot] = pltpu.bitcast(hist["mxu"][-1 - FENCE_LAG], U32)

    def tied(a):
        hist["n"] += 1
        if hist["due"] and hist["due"][0][0] <= hist["n"]:
            return jnp.where(never, hist["due"].pop(0)[1], a)
        if hist["n"] % TIE_EVERY == 0 and hist["vpu"]:
            live = hist["vpu"][-1]
            return jnp.where(never, live[(hist["n"] // TIE_EVERY) % len(live)], a)
        return a

    def mm(a, b, mask=None):
        a = tied(a)
        t = _mm(a if mask is None else jnp.where(mask, a, 0.0), b)
        hist["mxu"].append(t)
        return t

    def matvec(a, ref, g0, cols, out):
        for n, c in enumerate(cols):
            for kt, at in enumerate(a):
                t = mm(at, _tile(ref, g0 + kt * 8, c))
                out[n] = t if out[n] is None else out[n] + t
                yield 8

    def q_partial(xo, kt, i):
        q = [None] * 3 if kt == 0 else [qs[i, dt] for dt in range(3)]
        yield from matvec(xo, wqr, kt * 8, [i * 3 + dt for dt in range(3)], q)
        for dt in range(3):
            qs[i, dt] = q[dt]

    def q_finish(xo, coef, i):
        q = [qs[i, dt] for dt in range(3)]
        yield from matvec(xo, wqr, (ND - 1) * 8, [i * 3 + dt for dt in range(3)], q)
        for dt in range(3):
            qf[i, dt] = jnp.where(head_mask[dt], _rnd(_ln_apply(q[dt], coef)), 0.0)

    def softmax(i, buf, nc, meanwhile=()):
        q = [qf[i, dt] for dt in range(3)]
        m = None
        for j in range(NQ):
            s = None
            for sl in range(4):
                for dt in range(3):
                    t = mm(q[dt], _tile(kvr, i * GP + dt * 8, 4 * j + sl), slot_mask[sl])
                    s = t if s is None else s + t
                    yield 8
            ss[j] = s
            m = s if m is None else jnp.maximum(m, s)
        m = jnp.broadcast_to(jnp.max(m, axis=1, keepdims=True), (8, 128))
        m = jnp.maximum(m, pltpu.roll(m, 4, 0))
        m = jnp.maximum(m, pltpu.roll(m, 2, 0))
        yield from meanwhile
        l = None
        for j in range(NQ):
            p = jnp.exp2((ss[j] - m) * misc[SCALE])
            ps[buf][j] = p
            for c in range(4 * j, min(4 * j + 4, NKT - nc)):
                for hh in range(2):
                    r = (c % 4) * 2 + hh
                    pb[buf][pl.ds(c * 16 + hh, 8, stride=2), :] = jnp.broadcast_to(
                        p[r:r + 1], (8, 128))
            l = p if l is None else l + p
        ps[buf][NQ] = l

    def transpose_v(i, nc):
        def body(c, carry):
            for dt in range(3):
                g0 = (NP + i) * GP + dt * 8
                t = pltpu.bitcast(_tile(kvr, g0, c).T, U32)
                kvr[pl.ds(g0, 8), c] = t.reshape(8, 8, 128)
            return carry
        lax.fori_loop(NKT - nc, NKT, body, 0)

    def pv_vpu(i, buf, nc, side=()):
        side = iter(side)
        for hh in range(2):
            for gb in range(0, GP // 2, 2):
                yield next(side, 0)
                lo, hi = [None] * 2, [None] * 2
                for c in range(NKT - nc):
                    p = pb[buf][pl.ds(c * 16 + hh, 8, stride=2), :]
                    for g in range(2):
                        w = kvr[(NP + i) * GP + hh * (GP // 2) + gb + g, c]
                        a = pltpu.bitcast(w << 16, F32) * p
                        b = pltpu.bitcast(w & np.uint32(0xFFFF0000), F32) * p
                        lo[g] = a if lo[g] is None else lo[g] + a
                        hi[g] = b if hi[g] is None else hi[g] + b
                        yield 1.5
                    hist["vpu"].append(lo + hi)
                for g in range(2):
                    r0 = hh * DH + (gb + g) * 16
                    accs[buf][pl.ds(r0, 8, stride=2), :] = lo[g]
                    accs[buf][pl.ds(r0 + 1, 8, stride=2), :] = hi[g]

    def pv_mxu(i, buf, nc):
        om = [None] * 3
        for c in range(NKT - nc, NKT):
            p = _rnd(ps[buf][c // 4])
            for dt in range(3):
                t = mm(p, _tile(kvr, (NP + i) * GP + dt * 8, c), slot_mask[c % 4])
                om[dt] = t if om[dt] is None else om[dt] + t
                yield 8
        for dt in range(3):
            ps[buf][NQ + 1 + dt] = om[dt]

    def pv_finish(buf):
        l = _lane_sum([ps[buf][NQ]])
        l = l + pltpu.roll(l, 4, 0)
        l = l + pltpu.roll(l, 2, 0)
        inv = 1.0 / l
        inv_other = pltpu.roll(inv, 1, 0)
        for dt in range(3):
            t = accs[buf][pl.ds(dt * 128, 128), :].T.reshape(16, 8, 128)
            t = jnp.sum(t, axis=0) + jnp.where(head_mask[dt], ps[buf][NQ + 1 + dt], 0.0)
            t = _allsum_rows(t)
            o = _rnd(t * jnp.where(head_mask[dt], inv, inv_other))
            misc[OUT + dt] = o
            hist["due"].append((hist["n"] + FINISH_LAG, o))
            yield 8

    def out_proj(i):
        o = [misc[OUT + dt] for dt in range(3)]
        for c in range(ND):
            y = [ys[c]]
            yield from matvec(o, wor, i * GP, [c], y)
            ys[c] = y[0]

    def attention_streaming(x):
        reset()
        wait(first_copies)
        xo, (coef, rstd) = with_ones(x), _ln_stats(x, even)
        misc[SCALE] = rstd * EXP2_SCALE

        def prepare(i, carry):
            _run(q_partial(xo[:-1], 0, i), q_finish(xo[-1:], coef, i))
            transpose_v(i, jnp.where(i == NP - 1, MXU_TILES_LAST, MXU_TILES))
            return carry

        lax.fori_loop(0, NP, prepare, 0)
        wait(wo_copies)
        ys[...] = jnp.zeros(ys.shape, F32)

        def attend(i, nc):
            reset()
            _run(softmax(i, 0, nc), pv_mxu(i, 0, nc), pv_vpu(i, 0, nc), pv_finish(0))
            reset()
            _run(out_proj(i))

        def step(i, carry):
            for first, copies in zip(K_CUTS, k_copies[:-1]):
                pl.when(i == first)(functools.partial(wait, copies))
            attend(i, MXU_TILES)
            return carry

        lax.fori_loop(0, NP - 1, step, 0)
        wait(k_copies[-1])
        attend(NP - 1, MXU_TILES_LAST)
        return [ys[c] for c in range(ND)]

    def attention_resident(x):
        reset()
        accs[NB - 1][pl.ds(0, 2 * DH), :] = jnp.zeros((2 * DH, 128), F32)
        ps[NB - 1][NQ] = jnp.ones((8, 128), F32)
        ps[NB - 1][pl.ds(NQ + 1, 3)] = jnp.zeros((3, 8, 128), F32)
        ys[...] = jnp.zeros(ys.shape, F32)
        xo, (coef, rstd) = with_ones(x[-1:]), _ln_stats(x, even)
        misc[SCALE] = rstd * EXP2_SCALE
        q = [q_finish(xo, coef, i) for i in range(NP)]
        _run(*q[:3], softmax(0, 0, MXU_TILES, itertools.chain(*q[3:])))

        def step(t, carry):
            reset()
            mxu, vpu = [], []
            for u in range(NB):
                i = t * NB + u
                tail = itertools.chain(pv_mxu(i, u, MXU_TILES),
                                       out_proj(jnp.maximum(i - 1, 0)))
                mxu += [softmax(i + 1, (u + 1) % NB, MXU_TILES,
                                itertools.islice(tail, SOFTMAX_LAG)), tail]
                vpu += [pv_vpu(i, u, MXU_TILES, pv_finish((u - 1) % NB))]
            _interleave(itertools.chain(*mxu), itertools.chain(*vpu), RATIO, fence)
            return carry

        lax.fori_loop(0, (NP - 1) // NB, step, 0)
        reset()
        _interleave(
            itertools.chain(pv_mxu(NP - 1, 0, MXU_TILES_LAST), out_proj(NP - 2)),
            pv_vpu(NP - 1, 0, MXU_TILES_LAST, pv_finish(NB - 1)), RATIO_LAST, fence)
        _run(pv_finish(0))
        reset()
        _run(out_proj(NP - 1))
        return [ys[c] for c in range(ND)]

    def ffn_hidden(x, streaming):
        reset()
        xo, (coef, rstd) = with_ones(x), _ln_stats(x, even)
        coef = coef * rstd
        gate, up, h = [None] * NF, [None] * NF, []
        if streaming:
            wait(w1_copies)
            _run(matvec(xo, w1r, 0, range(NF), gate))
            wait(w3_copies)
            _run(matvec(xo, w3r, 0, range(NF), up))
        for ft in range(NF):
            g, u = gate[ft:ft + 1], up[ft:ft + 1]
            if not streaming:
                _run(matvec(xo, w1r, 0, [ft], g), matvec(xo, w3r, 0, [ft], u))
            g, u = _ln_apply(g[0], coef), _ln_apply(u[0], coef)
            h.append(_rnd(g / (1.0 + jnp.exp(-g)) * u))
        return h

    def add(x, y):
        return [_rnd(a + b) for a, b in zip(x, y)]

    x = add(x, attention_streaming(x))
    h = ffn_hidden(x, True)
    for c in range(ND):
        wait(w2_copies[c])
        f = [None]
        _run(matvec(h, w2r, 0, [c], f))
        x[c] = _rnd(x[c] + f[0])
        if c < ND - 1:
            xo = with_ones(x[c:c + 1])
            _run(*[q_partial(xo, c, i) for i in range(NP)])

    x = add(x, attention_resident(x))
    h = ffn_hidden(x, False)
    f = [None] * ND
    _run(*[matvec([h[kt]], w2r, kt * 8, range(ND), f) for kt in range(NF)])
    x = add(x, f)
    o_ref[...] = jnp.concatenate(x, axis=1)[0:1].astype(BF16)


def _tiles(a):
    r, c = a.shape
    return a.reshape(r // 16, 2, 8, c // 128, 128).transpose(0, 1, 3, 2, 4)


def _cache_tiles(a):
    a = a.reshape(H, SK // 128, 128, DH // 8, 8).transpose(0, 3, 1, 4, 2)
    return a.reshape(H * DH // 16, 2, SK // 128, 8, 128)


@jax.jit
def pallas_interleave_layers__sliding_block_cached__glu_gated_swiglu__decode_kernel(
    A_x: jax.Array,
    A_k_cache: jax.Array,
    A_v_cache: jax.Array,
    A_wq: jax.Array,
    A_wo: jax.Array,
    B_x: jax.Array,
    B_w1: jax.Array,
    B_w3: jax.Array,
    B_w2: jax.Array,
):
    del B_x
    out = pl.pallas_call(
        _kernel,
        out_shape=jax.ShapeDtypeStruct((1, D), BF16),
        in_specs=[pl.BlockSpec(memory_space=pl.ANY)] * 8,
        out_specs=pl.BlockSpec(memory_space=pltpu.VMEM),
        scratch_shapes=[
            pltpu.VMEM((2 * NP * GP + 1, NKT, 16, 128), BF16),
            pltpu.VMEM((D // 16, H * DH // 128, 16, 128), BF16),
            pltpu.VMEM((H * DH // 16, ND, 16, 128), BF16),
            pltpu.VMEM((D // 16, NF, 16, 128), BF16),
            pltpu.VMEM((D // 16, NF, 16, 128), BF16),
            pltpu.VMEM((FF // 16, ND, 16, 128), BF16),
            pltpu.VMEM((NP, 3, 8, 128), F32),
            pltpu.VMEM((NP, 3, 8, 128), F32),
            pltpu.VMEM((NQ, 8, 128), F32),
            pltpu.VMEM((ND, 8, 128), F32),
            pltpu.VMEM((4, 8, 128), F32),
            *[pltpu.VMEM((NQ + 4, 8, 128), F32)] * NB,
            *[pltpu.VMEM((NKT * 16, 128), F32)] * NB,
            *[pltpu.VMEM((2 * DH + 8, 128), F32)] * NB,
            pltpu.VMEM((1, D), BF16),
            pltpu.SemaphoreType.DMA((4 + len(K_CUTS) + ND,)),
        ],
        compiler_params=pltpu.CompilerParams(vmem_limit_bytes=124 * 1024 * 1024),
        name="fused",
    )(A_x.reshape(1, D), _cache_tiles(A_k_cache), _cache_tiles(A_v_cache),
      _tiles(A_wq), _tiles(A_wo), _tiles(B_w1), _tiles(B_w3), _tiles(B_w2))
    return out.reshape(1, 1, D)
```

```python
import functools
import itertools

import jax
import jax.numpy as jnp
import numpy as np
from jax import lax
import jax.experimental.pallas as pl
import jax.experimental.pallas.tpu as pltpu

F32, BF16, U32 = jnp.float32, jnp.bfloat16, jnp.uint32

D = 640
H = 32
DH = 192
SK = 32768
W = min(4096, max(256, SK // 4))
FF = 1536
EPS = 1e-5
EXP2_SCALE = float(DH ** -0.5 * np.log2(np.e))

NP = H // 2
GP = 2 * DH // 16
NKT = W // 128
NQ = NKT // 4
ND = D // 128
NF = FF // 128

NB = 3
MXU_TILES = 6
MXU_TILES_LAST = 20
K_CUTS = (0, 8, 12, 15, NP)
SCALE, OUT = 0, 1

RATIO, RATIO_LAST = 0.93, 1.0
FENCE_EVERY, FENCE_LAG = 128, 18
TIE_EVERY, FINISH_LAG, SOFTMAX_LAG = 2, 36, 20


def _mm(a, b):
    return lax.dot_general(a, b, (((1,), (0,)), ((), ())),
                           precision=lax.Precision.DEFAULT,
                           preferred_element_type=F32)


def _rnd(a):
    return a.astype(BF16).astype(F32)


def _tile(ref, g0, c):
    return pltpu.bitcast(ref[pl.ds(g0, 8), c].reshape(64, 128), BF16)


def _allsum_rows(a):
    a = a + pltpu.roll(a, 4, 0)
    a = a + pltpu.roll(a, 2, 0)
    return a + pltpu.roll(a, 1, 0)


def _lane_sum(tiles):
    s = jnp.sum(functools.reduce(jnp.add, tiles), axis=1, keepdims=True)
    return jnp.broadcast_to(s, (8, 128))


def _ln_stats(x, even):
    m = _lane_sum(x) * (1.0 / D)
    v = _lane_sum([(t - m) * (t - m) for t in x]) * (1.0 / D)
    return jnp.where(even, 1.0, -m), lax.rsqrt(v + EPS)


def _ln_apply(t, coef):
    t = t * coef
    return t + pltpu.roll(t, 1, 0)


def _run(*gens):
    for g in gens:
        for _ in g:
            pass


def _interleave(a, b, ratio, fence):
    end = object()
    ta = tb = 0.0
    nxt = FENCE_EVERY
    while a is not None or b is not None:
        if a is not None and b is not None and tb >= nxt:
            fence()
            nxt = tb + FENCE_EVERY
        if b is None or (a is not None and ta * ratio <= tb):
            c = next(a, end)
            if c is end:
                a = None
            else:
                ta += c
        else:
            c = next(b, end)
            if c is end:
                b = None
            else:
                tb += c


def _kernel(x_hbm, k_hbm, v_hbm, wq_hbm, wo_hbm, w1_hbm, w3_hbm, w2_hbm, o_ref,
            kb, vb, wqb, wob, w1b, w3b, w2b, qs, qf, ss, ys, misc, *rest):
    ps, pb, accs = rest[:NB], rest[NB:2 * NB], rest[2 * NB:3 * NB]
    xb, sems = rest[3 * NB:]
    kr, vr = kb.bitcast(U32), vb.bitcast(U32)
    wqr, wor = wqb.bitcast(U32), wob.bitcast(U32)
    w1r, w3r, w2r = w1b.bitcast(U32), w3b.bitcast(U32), w2b.bitcast(U32)

    def kv_copies(src, dst, i, n, slot):
        return [pltpu.make_async_copy(
            src.at[pl.ds(i * GP, n * GP), half, pl.ds((SK - W) // 128, NKT)],
            dst.at[pl.ds(i * GP, n * GP), :, pl.ds(half * 8, 8)],
            sems.at[slot]) for half in range(2)]

    def w_copies(src, dst, slot, c=slice(None)):
        return [pltpu.make_async_copy(
            src.at[:, half, c], dst.at[:, c, pl.ds(half * 8, 8)], sems.at[slot])
            for half in range(2)]

    def wait(copies):
        for c in copies:
            c.wait()

    x_copies = [pltpu.make_async_copy(x_hbm, xb, sems.at[0])]
    first_copies = w_copies(wq_hbm, wqb, 1) + kv_copies(v_hbm, vb, 0, NP, 1)
    wo_copies = w_copies(wo_hbm, wob, 2)
    k_copies = [kv_copies(k_hbm, kb, a, b - a, 3 + n)
                for n, (a, b) in enumerate(zip(K_CUTS, K_CUTS[1:]))]
    ns = 3 + len(k_copies)
    w1_copies, w3_copies = w_copies(w1_hbm, w1b, ns), w_copies(w3_hbm, w3b, ns + 1)
    w2_copies = [w_copies(w2_hbm, w2b, ns + 2 + c, c) for c in range(ND)]
    for c in itertools.chain(x_copies, first_copies, wo_copies, *k_copies,
                             w1_copies, w3_copies, *w2_copies):
        c.start()

    wait(x_copies)
    x = jnp.broadcast_to(xb[...].astype(F32), (8, D))
    x = [x[:, c * 128:(c + 1) * 128] for c in range(ND)]

    row = lax.broadcasted_iota(jnp.int32, (8, 128), 0)
    lane = lax.broadcasted_iota(jnp.int32, (8, 128), 1)
    head_of_lane = [jnp.zeros_like(lane), (lane >= 64).astype(jnp.int32),
                    jnp.ones_like(lane)]
    head_mask = [(row & 1) == h for h in head_of_lane]
    slot_mask = [(row >> 1) == s for s in range(4)]
    even = (row & 1) == 0

    def with_ones(x):
        return [jnp.where(even, t, 1.0) for t in x]

    spot = jnp.max(pltpu.bitcast(x[0], jnp.int32) & 1)
    never = lane == spot + 128
    hist = {}

    def reset():
        hist.update(vpu=[], mxu=[], due=[], n=0)

    def fence():
        if len(hist["mxu"]) > FENCE_LAG:
            vr[NP * GP, spot] = pltpu.bitcast(hist["mxu"][-1 - FENCE_LAG], U32)

    def tied(a):
        hist["n"] += 1
        if hist["due"] and hist["due"][0][0] <= hist["n"]:
            return jnp.where(never, hist["due"].pop(0)[1], a)
        if hist["n"] % TIE_EVERY == 0 and hist["vpu"]:
            live = hist["vpu"][-1]
            return jnp.where(never, live[(hist["n"] // TIE_EVERY) % len(live)], a)
        return a

    def mm(a, b, mask=None):
        a = tied(a)
        t = _mm(a if mask is None else jnp.where(mask, a, 0.0), b)
        hist["mxu"].append(t)
        return t

    def matvec(a, ref, g0, cols, out):
        for n, c in enumerate(cols):
            for kt, at in enumerate(a):
                t = mm(at, _tile(ref, g0 + kt * 8, c))
                out[n] = t if out[n] is None else out[n] + t
                yield 8

    def q_partial(xo, kt, i):
        q = [None] * 3 if kt == 0 else [qs[i, dt] for dt in range(3)]
        yield from matvec(xo, wqr, kt * 8, [i * 3 + dt for dt in range(3)], q)
        for dt in range(3):
            qs[i, dt] = q[dt]

    def q_finish(xo, coef, i):
        q = [qs[i, dt] for dt in range(3)]
        yield from matvec(xo, wqr, (ND - 1) * 8, [i * 3 + dt for dt in range(3)], q)
        for dt in range(3):
            qf[i, dt] = jnp.where(head_mask[dt], _rnd(_ln_apply(q[dt], coef)), 0.0)

    def softmax(i, buf, nc, meanwhile=()):
        q = [qf[i, dt] for dt in range(3)]
        m = None
        for j in range(NQ):
            s = None
            for sl in range(4):
                for dt in range(3):
                    t = mm(q[dt], _tile(kr, i * GP + dt * 8, 4 * j + sl), slot_mask[sl])
                    s = t if s is None else s + t
                    yield 8
            ss[j] = s
            m = s if m is None else jnp.maximum(m, s)
        m = jnp.broadcast_to(jnp.max(m, axis=1, keepdims=True), (8, 128))
        m = jnp.maximum(m, pltpu.roll(m, 4, 0))
        m = jnp.maximum(m, pltpu.roll(m, 2, 0))
        yield from meanwhile
        l = None
        for j in range(NQ):
            p = jnp.exp2((ss[j] - m) * misc[SCALE])
            ps[buf][j] = p
            for c in range(4 * j, min(4 * j + 4, NKT - nc)):
                for hh in range(2):
                    r = (c % 4) * 2 + hh
                    pb[buf][pl.ds(c * 16 + hh, 8, stride=2), :] = jnp.broadcast_to(
                        p[r:r + 1], (8, 128))
            l = p if l is None else l + p
        ps[buf][NQ] = l

    def transpose_v(i, nc):
        def body(c, carry):
            for dt in range(3):
                g0 = i * GP + dt * 8
                t = pltpu.bitcast(_tile(vr, g0, c).T, U32)
                vr[pl.ds(g0, 8), c] = t.reshape(8, 8, 128)
            return carry
        lax.fori_loop(NKT - nc, NKT, body, 0)

    def pv_vpu(i, buf, nc, side=()):
        side = iter(side)
        for hh in range(2):
            for gb in range(0, GP // 2, 2):
                yield next(side, 0)
                lo, hi = [None] * 2, [None] * 2
                for c in range(NKT - nc):
                    p = pb[buf][pl.ds(c * 16 + hh, 8, stride=2), :]
                    for g in range(2):
                        w = vr[i * GP + hh * (GP // 2) + gb + g, c]
                        a = pltpu.bitcast(w << 16, F32) * p
                        b = pltpu.bitcast(w & np.uint32(0xFFFF0000), F32) * p
                        lo[g] = a if lo[g] is None else lo[g] + a
                        hi[g] = b if hi[g] is None else hi[g] + b
                        yield 1.5
                    hist["vpu"].append(lo + hi)
                for g in range(2):
                    r0 = hh * DH + (gb + g) * 16
                    accs[buf][pl.ds(r0, 8, stride=2), :] = lo[g]
                    accs[buf][pl.ds(r0 + 1, 8, stride=2), :] = hi[g]

    def pv_mxu(i, buf, nc):
        om = [None] * 3
        for c in range(NKT - nc, NKT):
            p = _rnd(ps[buf][c // 4])
            for dt in range(3):
                t = mm(p, _tile(vr, i * GP + dt * 8, c), slot_mask[c % 4])
                om[dt] = t if om[dt] is None else om[dt] + t
                yield 8
        for dt in range(3):
            ps[buf][NQ + 1 + dt] = om[dt]

    def pv_finish(buf):
        l = _lane_sum([ps[buf][NQ]])
        l = l + pltpu.roll(l, 4, 0)
        l = l + pltpu.roll(l, 2, 0)
        inv = 1.0 / l
        inv_other = pltpu.roll(inv, 1, 0)
        for dt in range(3):
            t = accs[buf][pl.ds(dt * 128, 128), :].T.reshape(16, 8, 128)
            t = jnp.sum(t, axis=0) + jnp.where(head_mask[dt], ps[buf][NQ + 1 + dt], 0.0)
            t = _allsum_rows(t)
            o = _rnd(t * jnp.where(head_mask[dt], inv, inv_other))
            misc[OUT + dt] = o
            hist["due"].append((hist["n"] + FINISH_LAG, o))
            yield 8

    def out_proj(i):
        o = [misc[OUT + dt] for dt in range(3)]
        for c in range(ND):
            y = [ys[c]]
            yield from matvec(o, wor, i * GP, [c], y)
            ys[c] = y[0]

    def attention_streaming(x):
        reset()
        wait(first_copies)
        xo, (coef, rstd) = with_ones(x), _ln_stats(x, even)
        misc[SCALE] = rstd * EXP2_SCALE

        def prepare(i, carry):
            _run(q_partial(xo[:-1], 0, i), q_finish(xo[-1:], coef, i))
            transpose_v(i, jnp.where(i == NP - 1, MXU_TILES_LAST, MXU_TILES))
            return carry

        lax.fori_loop(0, NP, prepare, 0)
        wait(wo_copies)
        ys[...] = jnp.zeros(ys.shape, F32)

        def attend(i, nc):
            reset()
            _run(softmax(i, 0, nc), pv_mxu(i, 0, nc), pv_vpu(i, 0, nc), pv_finish(0))
            reset()
            _run(out_proj(i))

        def step(i, carry):
            for first, copies in zip(K_CUTS, k_copies[:-1]):
                pl.when(i == first)(functools.partial(wait, copies))
            attend(i, MXU_TILES)
            return carry

        lax.fori_loop(0, NP - 1, step, 0)
        wait(k_copies[-1])
        attend(NP - 1, MXU_TILES_LAST)
        return [ys[c] for c in range(ND)]

    def attention_resident(x):
        reset()
        accs[NB - 1][pl.ds(0, 2 * DH), :] = jnp.zeros((2 * DH, 128), F32)
        ps[NB - 1][NQ] = jnp.ones((8, 128), F32)
        ps[NB - 1][pl.ds(NQ + 1, 3)] = jnp.zeros((3, 8, 128), F32)
        ys[...] = jnp.zeros(ys.shape, F32)
        xo, (coef, rstd) = with_ones(x[-1:]), _ln_stats(x, even)
        misc[SCALE] = rstd * EXP2_SCALE
        q = [q_finish(xo, coef, i) for i in range(NP)]
        _run(*q[:3], softmax(0, 0, MXU_TILES, itertools.chain(*q[3:])))

        def step(t, carry):
            reset()
            mxu, vpu = [], []
            for u in range(NB):
                i = t * NB + u
                tail = itertools.chain(pv_mxu(i, u, MXU_TILES),
                                       out_proj(jnp.maximum(i - 1, 0)))
                mxu += [softmax(i + 1, (u + 1) % NB, MXU_TILES,
                                itertools.islice(tail, SOFTMAX_LAG)), tail]
                vpu += [pv_vpu(i, u, MXU_TILES, pv_finish((u - 1) % NB))]
            _interleave(itertools.chain(*mxu), itertools.chain(*vpu), RATIO, fence)
            return carry

        lax.fori_loop(0, (NP - 1) // NB, step, 0)
        reset()
        _interleave(
            itertools.chain(pv_mxu(NP - 1, 0, MXU_TILES_LAST), out_proj(NP - 2)),
            pv_vpu(NP - 1, 0, MXU_TILES_LAST, pv_finish(NB - 1)), RATIO_LAST, fence)
        _run(pv_finish(0))
        reset()
        _run(out_proj(NP - 1))
        return [ys[c] for c in range(ND)]

    def ffn_hidden(x, streaming):
        reset()
        xo, (coef, rstd) = with_ones(x), _ln_stats(x, even)
        coef = coef * rstd
        gate, up, h = [None] * NF, [None] * NF, []
        if streaming:
            wait(w1_copies)
            _run(matvec(xo, w1r, 0, range(NF), gate))
            wait(w3_copies)
            _run(matvec(xo, w3r, 0, range(NF), up))
        for ft in range(NF):
            g, u = gate[ft:ft + 1], up[ft:ft + 1]
            if not streaming:
                _run(matvec(xo, w1r, 0, [ft], g), matvec(xo, w3r, 0, [ft], u))
            g, u = _ln_apply(g[0], coef), _ln_apply(u[0], coef)
            h.append(_rnd(g / (1.0 + jnp.exp(-g)) * u))
        return h

    def add(x, y):
        return [_rnd(a + b) for a, b in zip(x, y)]

    x = add(x, attention_streaming(x))
    h = ffn_hidden(x, True)
    for c in range(ND):
        wait(w2_copies[c])
        f = [None]
        _run(matvec(h, w2r, 0, [c], f))
        x[c] = _rnd(x[c] + f[0])
        if c < ND - 1:
            xo = with_ones(x[c:c + 1])
            _run(*[q_partial(xo, c, i) for i in range(NP)])

    x = add(x, attention_resident(x))
    h = ffn_hidden(x, False)
    f = [None] * ND
    _run(*[matvec([h[kt]], w2r, kt * 8, range(ND), f) for kt in range(NF)])
    x = add(x, f)
    o_ref[...] = jnp.concatenate(x, axis=1)[0:1].astype(BF16)


def _tiles(a):
    r, c = a.shape
    return a.reshape(r // 16, 2, 8, c // 128, 128).transpose(0, 1, 3, 2, 4)


def _cache_tiles(a):
    a = a.reshape(H, SK // 128, 128, DH // 8, 8).transpose(0, 3, 1, 4, 2)
    return a.reshape(H * DH // 16, 2, SK // 128, 8, 128)


@jax.jit
def pallas_interleave_layers__sliding_block_cached__glu_gated_swiglu__decode_kernel(
    A_x: jax.Array,
    A_k_cache: jax.Array,
    A_v_cache: jax.Array,
    A_wq: jax.Array,
    A_wo: jax.Array,
    B_x: jax.Array,
    B_w1: jax.Array,
    B_w3: jax.Array,
    B_w2: jax.Array,
):
    del B_x
    out = pl.pallas_call(
        _kernel,
        out_shape=jax.ShapeDtypeStruct((1, D), BF16),
        in_specs=[pl.BlockSpec(memory_space=pl.ANY)] * 8,
        out_specs=pl.BlockSpec(memory_space=pltpu.VMEM),
        scratch_shapes=[
            pltpu.VMEM((NP * GP, NKT, 16, 128), BF16),
            pltpu.VMEM((NP * GP + 1, NKT, 16, 128), BF16),
            pltpu.VMEM((D // 16, H * DH // 128, 16, 128), BF16),
            pltpu.VMEM((H * DH // 16, ND, 16, 128), BF16),
            pltpu.VMEM((D // 16, NF, 16, 128), BF16),
            pltpu.VMEM((D // 16, NF, 16, 128), BF16),
            pltpu.VMEM((FF // 16, ND, 16, 128), BF16),
            pltpu.VMEM((NP, 3, 8, 128), F32),
            pltpu.VMEM((NP, 3, 8, 128), F32),
            pltpu.VMEM((NQ, 8, 128), F32),
            pltpu.VMEM((ND, 8, 128), F32),
            pltpu.VMEM((4, 8, 128), F32),
            *[pltpu.VMEM((NQ + 4, 8, 128), F32)] * NB,
            *[pltpu.VMEM((NKT * 16, 128), F32)] * NB,
            *[pltpu.VMEM((2 * DH + 8, 128), F32)] * NB,
            pltpu.VMEM((1, D), BF16),
            pltpu.SemaphoreType.DMA((4 + len(K_CUTS) + ND,)),
        ],
        compiler_params=pltpu.CompilerParams(vmem_limit_bytes=124 * 1024 * 1024),
        name="fused",
    )(A_x.reshape(1, D), _cache_tiles(A_k_cache), _cache_tiles(A_v_cache),
      _tiles(A_wq), _tiles(A_wo), _tiles(B_w1), _tiles(B_w3), _tiles(B_w2))
    return out.reshape(1, 1, D)
```
